```python
import jax
import jax.numpy as jnp

def _softmax(x, axis=-1):
    return jax.nn.softmax(x, axis=axis)

def _gelu(x):
    return jax.nn.gelu(x, approximate=True)

def _silu(x):
    return jax.nn.silu(x)

def _sigmoid(x):
    return jax.nn.sigmoid(x)

def _layernorm(x, axis=-1, eps=1e-05):
    m = jnp.mean(x, axis=axis, keepdims=True)
    v = jnp.var(x, axis=axis, keepdims=True)
    return (x - m) / jnp.sqrt(v + eps)

def _scatter_add(tgt, idx, src, axis=0):
    return tgt.at[idx].add(src)

def _segment_sum(src, seg, n):
    return jax.ops.segment_sum(src, seg, n)

class _Rng:

    def __init__(self, key):
        self._k = key

    def _next(self):
        self._k, sub = jax.random.split(self._k)
        return sub

    def normal(self, shape):
        return jax.random.normal(self._next(), shape, dtype=jnp.bfloat16)

    def randint(self, lo, hi, shape):
        return jax.random.randint(self._next(), shape, lo, hi, dtype=jnp.int32)

    def uniform(self, shape, lo=0.0, hi=1.0):
        return jax.random.uniform(self._next(), shape, jnp.bfloat16, lo, hi)

    def permutation(self, n):
        return jax.random.permutation(self._next(), n)
kernel_name = 'adaLN_cond__sliding_local_dilated__glu_gated_swiglu__prompt'

def setup_inputs():
    _rng = _Rng(jax.random.key(int.from_bytes(__import__("os").urandom(4), "little")))
    _w = lambda a: (lambda t: t.astype(jnp.bfloat16) if jnp.issubdtype(t.dtype, jnp.floating) else t)(jnp.asarray(a))

    def _A_setup():
        B, S, D = (1, 2048, 1024)
        return {'x': _w((lambda *s: _rng.normal(s) * 0.05)(B, S, D)), 'wqkv': _w((lambda *s: _rng.normal(s) * 0.05)(D, 3 * D)), 'wo': _w((lambda *s: _rng.normal(s) * 0.05)(D, D))}
    _A_in = _A_setup()

    def _B_setup():
        B, S, D, F = (1, 2048, 1024, 3584)
        return {'x': _w((lambda *s: _rng.normal(s) * 0.05)(B, S, D)), 'w1': _w((lambda *s: _rng.normal(s) * 0.05)(D, F) * (2.0 / D) ** 0.5), 'w3': _w((lambda *s: _rng.normal(s) * 0.05)(D, F) * (2.0 / D) ** 0.5), 'w2': _w((lambda *s: _rng.normal(s) * 0.05)(F, D) * (2.0 / F) ** 0.5)}
    _B_in = _B_setup()
    return {'A_x': _A_in['x'], 'A_wqkv': _A_in['wqkv'], 'A_wo': _A_in['wo'], 'B_x': _B_in['x'], 'B_w1': _B_in['w1'], 'B_w3': _B_in['w3'], 'B_w2': _B_in['w2'], 'c': _w((lambda *s: _rng.normal(s) * 0.05)(1, 1024)), 'w_mod': _w((lambda *s: _rng.normal(s) * 0.05)(1024, 6 * 1024) * 1024 ** (-0.5))}

def reference(A_x, A_wqkv, A_wo, B_x, B_w1, B_w3, B_w2, c, w_mod):

    def _A_ref(x, wqkv, wo):
        B, S, D = x.shape
        H = 32
        Dh = D // H
        W, dil = (8, 2)
        qkv = (lambda x, *d: x.transpose(*d))((x @ wqkv).reshape(B, S, 3, H, Dh), 2, 0, 3, 1, 4)
        q, k, v = (qkv[0], qkv[1], qkv[2])
        scale = Dh ** (-0.5)
        pos = jnp.arange(S)
        off = jnp.arange(W) * dil
        idx = pos[:, None] - off[None, :]
        mask = idx >= 0
        idx_c = jnp.where(mask, idx, 0).reshape(-1)
        kg = k[:, :, idx_c, :].reshape(B, H, S, W, Dh)
        vg = v[:, :, idx_c, :].reshape(B, H, S, W, Dh)
        logits = jnp.einsum('bhsd,bhswd->bhsw', q, kg) * scale
        logits = jnp.where(mask[None, None, :, :], logits, -1000000000.0)
        attn = _softmax(logits, axis=-1)
        o = jnp.einsum('bhsw,bhswd->bhsd', attn, vg)
        return (lambda x, *d: x.transpose(*d))(o, 0, 2, 1, 3).reshape(B, S, D) @ wo

    def _B_ref(x, w1, w3, w2):
        gate = jnp.einsum('bsd,df->bsf', x, w1)
        up = jnp.einsum('bsd,df->bsf', x, w3)
        h = _silu(gate) * up
        out = jnp.einsum('bsf,fd->bsd', h, w2)
        return out
    x = A_x
    mod = (_silu(c) @ w_mod).reshape(c.shape[0], 6, 1, -1)
    sa, ca, ga, sb, cb, gb = (mod[:, 0].copy(), mod[:, 1].copy(), mod[:, 2].copy(), mod[:, 3].copy(), mod[:, 4].copy(), mod[:, 5].copy())
    h = _layernorm(x, axis=-1) * (1 + ca) + sa
    x = x + ga * _A_ref(h, A_wqkv, A_wo)
    h = _layernorm(x, axis=-1) * (1 + cb) + sb
    x = x + gb * _B_ref(h, B_w1, B_w3, B_w2)
    return x
```

```python
import functools

import jax
import jax.numpy as jnp
from jax import lax
import jax.experimental.pallas as pl
import jax.experimental.pallas.tpu as pltpu

S, D, H, DH, F = 2048, 1024, 32, 32, 3584
W, DIL = 8, 2
HALO = 16
EPS = 1e-5
LOG2E = 1.4426950408889634
NSL = D // 128
F32, BF16, U32, I32 = jnp.float32, jnp.bfloat16, jnp.uint32, jnp.int32

TM = 256
RB = 16
FC = 512
LNB = 32
T0 = 640
N1 = 4
T1 = (S - T0) // N1
KCHUNKS = (256, 256, 512)
NT = S // TM
NF = F // FC
NBLK = TM // RB
NB1 = NBLK // N1
SCHED = [NBLK // NF + (1 if f < NBLK % NF else 0) for f in range(NF)]


def _butterfly(xs):
    lane = lax.broadcasted_iota(I32, xs[0].shape, 1)
    for b in (4, 2, 1):
        m = (lane & b) != 0
        ys = list(xs)
        for j in range(8):
            if j & b == 0:
                lo, hi = xs[j], xs[j | b]
                ys[j] = jnp.where(m, pltpu.roll(hi, b, 1), lo)
                ys[j | b] = jnp.where(m, hi, pltpu.roll(lo, 128 - b, 1))
        xs = ys
    return xs


def _ln_norm(xf):
    m = jnp.mean(xf, axis=-1, keepdims=True)
    xc = xf - m
    v = jnp.mean(xc * xc, axis=-1, keepdims=True)
    return xc * lax.rsqrt(v + EPS)


def _bf(u):
    return pltpu.bitcast(u, BF16)


def _u32(b):
    return pltpu.bitcast(b, U32)


def _mo(v, m):
    return v if isinstance(v, int) else pl.multiple_of(v, m)


def _kernel(x_h, c_h, wqkv_h, wo_h, w1_h, w3_h, w2_h, wm_h, o_h,
            x_v, c_v, wqkv_v, wo_v, w1_v, w3_v, w2_v, wm_v, mod_v,
            qraw, kbuf, vbuf, hbuf, obuf, o_v, sems, osem):
    wqkv_u, wo_u, w1_u, w3_u, w2_u, wm_u = [
        r.bitcast(U32) for r in (wqkv_h, wo_h, w1_h, w3_h, w2_h, wm_h)]
    mac = pltpu.make_async_copy

    cp_c = mac(c_h, c_v, sems.at[0])
    cp_x0 = mac(x_h.at[0:T0, :], x_v.at[0:T0, :], sems.at[1])
    cp_xn = mac(x_h.at[T0:T0 + T1, :], x_v.at[T0:T0 + T1, :], sems.at[2])
    cp_xr = mac(x_h.at[T0 + T1:S, :], x_v.at[T0 + T1:S, :], sems.at[3])
    cp_wm = [mac(wm_u.at[:, j * D:(j + 1) * D], wm_v.at[j], sems.at[4 + j]) for j in range(6)]
    kcs, o = [], 0
    for n, wdt in enumerate(KCHUNKS):
        kcs.append(mac(wqkv_u.at[:, D + o:D + o + wdt], wqkv_v.at[:, D + o:D + o + wdt], sems.at[16 + n]))
        o += wdt
    cp_wv = mac(wqkv_u.at[:, 2 * D:3 * D], wqkv_v.at[:, 2 * D:3 * D], sems.at[10])
    cp_wq = mac(wqkv_u.at[:, 0:D], wqkv_v.at[:, 0:D], sems.at[11])
    cp_wo = mac(wo_u, wo_v, sems.at[12])
    cp_w1 = mac(w1_u, w1_v, sems.at[13])
    cp_w3 = mac(w3_u, w3_v, sems.at[14])
    cp_w2 = mac(w2_u, w2_v, sems.at[15])
    for cp in ([cp_c, cp_x0, cp_wm[0], cp_wm[1]] + kcs
               + [cp_wv, cp_xn, cp_wq, cp_xr, cp_wm[2], cp_wm[3], cp_wm[4], cp_wm[5],
                  cp_wo, cp_w1, cp_w3, cp_w2]):
        cp.start()

    kbuf[:, 0:HALO, :] = jnp.zeros((NSL, HALO, 128), F32)
    vbuf[:, 0:HALO, :] = jnp.zeros((NSL, HALO, 128), F32)
    cp_c.wait()
    cf = c_v[...].astype(F32)
    sc = jnp.broadcast_to((cf * jax.nn.sigmoid(cf)).astype(BF16), (16, D))

    def do_mod(j):
        r = jnp.dot(sc, _bf(wm_v[j]), preferred_element_type=F32)
        if j in (1, 4):
            r = 1.0 + r
        mod_v[j] = r

    def mod(j):
        return mod_v[j, 0:1, :]

    def ln1(r0, rows):
        outs = []
        for b in range(rows // LNB):
            xf = x_v[pl.ds(r0 + b * LNB, LNB), :].astype(F32)
            outs.append((_ln_norm(xf) * mod(1) + mod(0)).astype(BF16))
        return jnp.concatenate(outs, axis=0)

    def proj(h, t, cols=(0, D)):
        y = jnp.dot(h, _bf(wqkv_v[:, t * D + cols[0]:t * D + cols[1]]), preferred_element_type=F32)
        if t == 0:
            y = y * (DH ** -0.5 * LOG2E)
        return y

    def store_q(r0, y):
        qraw[pl.ds(_mo(r0 // 2, 8), y.shape[0] // 2), :] = _u32(y.astype(BF16))

    def store_kv(buf, r0, y):
        rows = y.shape[0]
        yb = _u32(y.astype(BF16))
        ys = _butterfly([yb[:, j * 128:(j + 1) * 128] for j in range(NSL)])
        for j in range(NSL):
            buf[j, pl.ds(r0 + HALO, rows), :] = _bf(ys[j]).astype(F32)

    def attn_block(rr, masked):
        lane = lax.broadcasted_iota(I32, (RB, 128), 1)
        i16 = lane ^ 16
        i8 = lane ^ 8
        qh = _mo(rr // 2, RB // 2)
        qr = qraw[pl.ds(qh, RB // 2), :]
        q = _butterfly([qr[:, j * 128:(j + 1) * 128] for j in range(NSL)])
        q = [_bf(u).astype(F32) for u in q]
        lg = []
        for w in range(W):
            acc = None
            for j in range(NSL):
                t = q[j] * kbuf[j, pl.ds(rr + HALO - DIL * w, RB), :]
                acc = t if acc is None else acc + t
            acc = acc + jnp.take_along_axis(acc, i16, axis=1)
            acc = acc + jnp.take_along_axis(acc, i8, axis=1)
            if w > 0 and masked:
                pos = rr + lax.broadcasted_iota(I32, (RB, 128), 0)
                acc = jnp.where(pos >= DIL * w, acc, -1e9 * LOG2E)
            lg.append(acc)
        mx = functools.reduce(jnp.maximum, lg)
        es = [jnp.exp2(l - mx) for l in lg]
        z = functools.reduce(lambda a, b: a + b, es)
        rz = 1.0 / z
        ps = [e * rz for e in es]
        os_ = []
        for j in range(NSL):
            acc = None
            for w in range(W):
                t = ps[w] * vbuf[j, pl.ds(rr + HALO - DIL * w, RB), :]
                acc = t if acc is None else acc + t
            os_.append(acc)
        ob = _butterfly([_u32(u.astype(BF16)) for u in os_])
        obuf[pl.ds(qh, RB // 2), :] = jnp.concatenate(ob, axis=1)

    cp_x0.wait()
    xn = [_ln_norm(x_v[b * LNB:(b + 1) * LNB, :].astype(F32)) for b in range(T0 // LNB)]
    cp_wm[0].wait()
    do_mod(0)
    cp_wm[1].wait()
    do_mod(1)
    kcs[0].wait()
    h = jnp.concatenate([(u * mod(1) + mod(0)).astype(BF16) for u in xn], axis=0)
    yk, o = [], 0
    for n, wdt in enumerate(KCHUNKS):
        if n > 0:
            kcs[n].wait()
        yk.append(proj(h, 1, (o, o + wdt)))
        o += wdt
    yk = jnp.concatenate(yk, axis=1)
    cp_wv.wait()
    yv = proj(h, 2)
    store_kv(kbuf, 0, yk)
    cp_xn.wait()
    cp_wq.wait()
    hbuf[...] = _u32(ln1(T0, T1))
    yq = proj(h, 0)
    store_kv(vbuf, 0, yv)
    store_q(0, yq)
    cp_xr.wait()

    def body_a(i, carry):
        r0 = pl.multiple_of(T0 + i * T1, 16)
        rn = pl.multiple_of(jnp.minimum(T0 + (i + 1) * T1, S - T1), 16)

        def att(b):
            attn_block(pl.multiple_of((i * NB1 + b) * RB, RB), True)

        yk = proj(_bf(hbuf[...]), 1)
        att(0)
        store_kv(kbuf, r0, yk)
        yv = proj(_bf(hbuf[...]), 2)
        att(1)
        store_kv(vbuf, r0, yv)
        hn = ln1(rn, T1)
        yq = proj(_bf(hbuf[...]), 0)
        att(2)
        att(3)
        store_q(r0, yq)
        hbuf[...] = _u32(hn)
        return carry

    lax.fori_loop(0, N1, body_a, 0)

    for j in range(2, 6):
        cp_wm[j].wait()
    cp_wo.wait()
    cp_w1.wait()
    cp_w3.wait()
    cp_w2.wait()
    for j in range(2, 6):
        do_mod(j)

    hm = TM // 2

    def out_copy(r0):
        return mac(o_v.at[pl.ds(r0, TM), :], o_h.at[pl.ds(r0, TM), :], osem)

    def body_b(i, carry):
        r0 = pl.multiple_of(i * TM, TM)
        rn = pl.multiple_of(jnp.minimum(i + 1, NT - 1) * TM, TM)
        rh = pl.multiple_of(i * (TM // 2), TM // 2)
        x1s, h2s = [], []
        for s in range(2):
            ob = _bf(obuf[pl.ds(rh + s * (hm // 2), hm // 2), :])
            a = jnp.dot(ob, _bf(wo_v[...]), preferred_element_type=F32)
            x1 = x_v[pl.ds(r0 + s * hm, hm), :].astype(F32) + mod(2) * a
            x1s.append(x1)
            h2s.append((_ln_norm(x1) * mod(4) + mod(3)).astype(BF16))
        h2 = jnp.concatenate(h2s, axis=0)

        def gated(hh, fs):
            g = jnp.dot(hh, _bf(w1_v[:, fs]), preferred_element_type=F32)
            u = jnp.dot(hh, _bf(w3_v[:, fs]), preferred_element_type=F32)
            return (g * jax.nn.sigmoid(g) * u).astype(BF16)

        acc = None
        blk = 0
        for f in range(NF):
            fs = slice(f * FC, (f + 1) * FC)
            if f == 0:
                act = jnp.concatenate([gated(hh, fs) for hh in h2s], axis=0)
            else:
                act = gated(h2, fs)
            for _ in range(SCHED[f]):
                attn_block(pl.multiple_of(rn + blk * RB, RB), False)
                blk += 1
            t = jnp.dot(act, _bf(w2_v[f * FC // 2:(f + 1) * FC // 2, :]), preferred_element_type=F32)
            acc = t if acc is None else acc + t
        x1 = jnp.concatenate(x1s, axis=0)
        o_v[pl.ds(r0, TM), :] = (x1 + mod(5) * acc).astype(BF16)
        out_copy(r0).start()
        return carry

    lax.fori_loop(0, NT, body_b, 0)
    for i in range(NT):
        out_copy(i * TM).wait()


@jax.jit
def pallas_adaLN_cond__sliding_local_dilated__glu_gated_swiglu__prompt_kernel(
    A_x: jax.Array,
    A_wqkv: jax.Array,
    A_wo: jax.Array,
    B_x: jax.Array,
    B_w1: jax.Array,
    B_w3: jax.Array,
    B_w2: jax.Array,
    c: jax.Array,
    w_mod: jax.Array,
):
    del B_x
    anyspec = pl.BlockSpec(memory_space=pl.ANY)
    out = pl.pallas_call(
        _kernel,
        in_specs=[anyspec] * 8,
        out_specs=anyspec,
        out_shape=jax.ShapeDtypeStruct((S, D), BF16),
        scratch_shapes=[
            pltpu.VMEM((S, D), BF16),
            pltpu.VMEM((1, D), BF16),
            pltpu.VMEM((D // 2, 3 * D), U32),
            pltpu.VMEM((D // 2, D), U32),
            pltpu.VMEM((D // 2, F), U32),
            pltpu.VMEM((D // 2, F), U32),
            pltpu.VMEM((F // 2, D), U32),
            pltpu.VMEM((6, D // 2, D), U32),
            pltpu.VMEM((6, 16, D), F32),
            pltpu.VMEM((S // 2, D), U32),
            pltpu.VMEM((NSL, S + HALO, 128), F32),
            pltpu.VMEM((NSL, S + HALO, 128), F32),
            pltpu.VMEM((T1 // 2, D), U32),
            pltpu.VMEM((S // 2, D), U32),
            pltpu.VMEM((S, D), BF16),
            pltpu.SemaphoreType.DMA((16 + len(KCHUNKS),)),
            pltpu.SemaphoreType.DMA(()),
        ],
        compiler_params=pltpu.CompilerParams(vmem_limit_bytes=120 * 1024 * 1024),
    )(A_x.reshape(S, D), c, A_wqkv, A_wo, B_w1, B_w3, B_w2, w_mod)
    return out.reshape(1, S, D)
```

```python
import functools
import jax, jax.numpy as jnp
from jax import lax
from jax.experimental import pallas as pl
from jax.experimental.pallas import tpu as pltpu

S, D, H, DH, F = 2048, 1024, 32, 32, 3584
W, DIL = 8, 2
HALO = 16
EPS = 1e-5
LOG2E = 1.4426950408889634
NSL = D // 128
F32, BF16, U32 = jnp.float32, jnp.bfloat16, jnp.uint32


def butterfly(xs):
    lane = lax.broadcasted_iota(jnp.int32, xs[0].shape, 1)
    for b in (4, 2, 1):
        m = (lane & b) != 0
        ys = list(xs)
        for j in range(8):
            if j & b == 0:
                A, B = xs[j], xs[j | b]
                ys[j] = jnp.where(m, pltpu.roll(B, b, 1), A)
                ys[j | b] = jnp.where(m, B, pltpu.roll(A, 128 - b, 1))
        xs = ys
    return xs


def s_combos(a11, a12, a21, a22):
    s1 = a21 + a22
    s2 = s1 - a11
    s3 = a11 - a21
    s4 = a12 - s2
    return [a11, a12, s4, a22, s1, s2, s3]


def c_combos(p):
    p1, p2, p3, p4, p5, p6, p7 = p
    u2 = p1 + p6
    u3 = u2 + p7
    u4 = u2 + p5
    return (p1 + p2, u4 + p3, u3 - p4, u3 + p5)


def make(tm=256, rb=16, fc=512, lnb=32, sched=None, split0=True, t0=640, kchunks=(256, 256, 512),
         seq1="K,a0,sk,V,a1,sv,L,Q,a2,a3,sq,h", modmode="mid", nodma=False, xp=None, f_order=0, hsplit=2, late=0, stop=None, vshift='', satrick=True, sepbias=True, mdep='K', n1run=4, n2run=8, n1b=4, sn=256, prerb=16, precb=256):
    nt = S // tm
    nf = F // fc
    nblk = tm // rb
    n1 = 4
    t1 = (S - t0) // n1
    assert t0 + n1 * t1 == S and t1 % 16 == 0 and t1 % lnb == 0 and t0 % lnb == 0
    nb1 = n1b
    ntot = S // rb
    n2b = max(-(-(ntot - n1 * n1b) // (nt - 1)), 0)
    assert n1 * n1b >= nblk
    assert all(n1 * n1b + i * n2b >= nblk * (i + 1) for i in range(nt)) or n1 * n1b + (nt - 1) * n2b >= ntot
    if sched is None:
        base = n2b // nf; rem = n2b % nf
        sched = [base + (1 if f < rem else 0) for f in range(nf)]
    assert sum(sched) == n2b

    def ln_norm(xf):
        m = jnp.mean(xf, axis=-1, keepdims=True)
        xc = xf - m
        v = jnp.mean(xc * xc, axis=-1, keepdims=True)
        return xc * lax.rsqrt(v + EPS)

    class _Nop:
        def start(self): pass
        def wait(self): pass

    def mac(a, b, sem):
        return _Nop() if nodma else pltpu.make_async_copy(a, b, sem)

    def mo(v, m):
        return v if isinstance(v, int) else pl.multiple_of(v, m)

    def mn(a, b):
        return min(a, b) if isinstance(a, int) else jnp.minimum(a, b)

    def bf(u):
        return pltpu.bitcast(u, BF16)

    def u32(b):
        return pltpu.bitcast(b, U32)

    def kernel(x_h, c_h, wqkv_h, wo_h, w1_h, w3_h, w2_h, wm_h, o_h,
               x_v, c_v, wqkv_v, wo_v, w1_v, w3_v, w2_v, wm_v, mod_v, qraw, kbuf, vbuf, hbuf, obuf, o_v, bias_v, hf, scol, sems, osem):
        wqkv_u, wo_u, w1_u, w3_u, w2_u, wm_u = [r.bitcast(U32) for r in (wqkv_h, wo_h, w1_h, w3_h, w2_h, wm_h)]
        cp_c = mac(c_h, c_v, sems.at[0])
        cp_x0 = mac(x_h.at[0:t0, :], x_v.at[0:t0, :], sems.at[1])
        cp_xn = mac(x_h.at[t0:t0 + t1, :], x_v.at[t0:t0 + t1, :], sems.at[2])
        cp_xr = mac(x_h.at[t0 + t1:S, :], x_v.at[t0 + t1:S, :], sems.at[3])
        cp_wm = [mac(wm_u.at[:, j * D:(j + 1) * D], wm_v.at[j], sems.at[4 + j]) for j in range(6)]
        kcs, o = [], 0
        for n, w_ in enumerate(kchunks):
            kcs.append(mac(wqkv_u.at[:, D + o:D + o + w_], wqkv_v.at[:, D + o:D + o + w_], sems.at[16 + n])); o += w_
        assert o == D
        cp_wv = mac(wqkv_u.at[:, 2 * D:3 * D], wqkv_v.at[:, 2 * D:3 * D], sems.at[10])
        cp_wq = mac(wqkv_u.at[:, 0:D], wqkv_v.at[:, 0:D], sems.at[11])
        cp_wo = mac(wo_u, wo_v, sems.at[12])
        NS0 = 16 + len(kchunks)
        def wcopies(src, dst, kh, nh, base):
            return [mac(src.at[0:kh, 0:nh], dst.at[0], sems.at[base]),
                    mac(src.at[kh:2 * kh, 0:nh], dst.at[1], sems.at[base + 1]),
                    mac(src.at[kh:2 * kh, nh:2 * nh], dst.at[2], sems.at[base + 2]),
                    mac(src.at[0:kh, nh:2 * nh], dst.at[4], sems.at[base + 3])]
        cp_w1 = wcopies(w1_u, w1_v, D // 4, F // 2, NS0)
        cp_w3 = wcopies(w3_u, w3_v, D // 4, F // 2, NS0 + 4)
        cp_w2 = wcopies(w2_u, w2_v, F // 4, D // 2, NS0 + 8)
        early = [cp_c, cp_x0, cp_wm[1]] + kcs + [cp_wm[0], cp_wv, cp_xn, cp_wq, cp_xr]
        rest = [cp_wm[2], cp_wm[3], cp_wm[4], cp_wm[5], cp_wo] + cp_w1 + cp_w3 + cp_w2
        for cp in early + ([] if late else rest):
            cp.start()

        kbuf[:, 0:HALO, :] = jnp.zeros((NSL, HALO, 128), F32)
        vbuf[:, 0:HALO, :] = jnp.zeros((NSL, HALO, 128), F32)
        cp_c.wait()
        waited_c = True
        cf = c_v[...].astype(F32)
        sc = (cf * jax.nn.sigmoid(cf)).astype(BF16)
        if modmode == 'vpu':
            scol[...] = jnp.broadcast_to(sc.astype(F32), (128, D)).T
        sc = jnp.broadcast_to(sc, (16, D))

        def do_mod(j):
            r = jnp.dot(sc, bf(wm_v[j]), preferred_element_type=F32)
            if j in (1, 4):
                r = 1.0 + r
            mod_v[j] = r

        def do_mod_vpu(j, ydep):
            flag = kbuf[0, 0:8, :] != 0.0
            flag = jnp.concatenate([flag] * 2, axis=0)
            tot = None
            for p in range(8):
                accs = [None] * NSL
                for kb in range(8):
                    lo = p * 128 + kb * 16
                    sc_ = scol[lo:lo + 16, :]
                    if ydep is not None:
                        sc_ = jnp.where(flag, ydep[0:16, p * 128:(p + 1) * 128], sc_)
                    w = bf(wm_v[j, lo // 2:lo // 2 + 8, :]).astype(F32)
                    for jj in range(NSL):
                        t = w[:, jj * 128:(jj + 1) * 128] * sc_
                        t = t[0:8] + t[8:16]
                        accs[jj] = t if accs[jj] is None else accs[jj] + t
                r = jnp.concatenate(accs, axis=1)
                tot = r if tot is None else tot + r
            r = jnp.sum(tot, axis=0, keepdims=True) + jnp.where(j == 4, 1.0, 0.0)
            mod_v[j, 0:1, :] = r

        def mod(j):
            return mod_v[j, 0:1, :]

        def ln1(r0, rows):
            outs = []
            for b in range(rows // lnb):
                xf = x_v[pl.ds(r0 + b * lnb, lnb), :].astype(F32)
                outs.append((ln_norm(xf) * mod(1)).astype(BF16))
            return jnp.concatenate(outs, axis=0)

        bufs = [None, kbuf, vbuf]

        QS = DH ** -0.5 * LOG2E
        def a1_dot(h, t, cols=None, first=False):
            lo, hi = (0, D) if cols is None else cols
            wv_ = bf(wqkv_v[:, t * D + lo:t * D + hi])
            if t == 1:
                return jnp.dot(h, wv_, preferred_element_type=F32)
            if first and sepbias:
                b = jnp.dot(mod_v[0].astype(BF16), wv_, preferred_element_type=F32)[0:8, :]
                if t == 0:
                    b = b * QS
                bias_v[t // 2] = b
                b = b[0:1, :]
                y = jnp.dot(bf(hf[0:t0 // 2, :]), wv_, preferred_element_type=F32)
            elif first:
                rows = t0
                y = jnp.dot(bf(hf[...]), wv_, preferred_element_type=F32)
                b = y[rows:rows + 8, :]
                if t == 0:
                    b = b * QS
                bias_v[t // 2] = b
                y = y[0:rows, :]
                b = b[0:1, :]
            else:
                y = jnp.dot(h, wv_, preferred_element_type=F32)
                b = bias_v[t // 2, 0:1, :]
            return (y * QS + b) if t == 0 else (y + b)

        def a1_store(r0, t, y):
            rows = y.shape[0]
            yb = u32(y.astype(BF16))
            if t == 0:
                qraw[pl.ds(mo(r0 // 2, 8), rows // 2), :] = yb
            else:
                ys = butterfly([yb[:, j * 128:(j + 1) * 128] for j in range(NSL)])
                for j in range(NSL):
                    bufs[t][j, pl.ds(r0 + HALO, rows), :] = bf(ys[j]).astype(F32)

        def attn_block(rr, masked):
            lane = lax.broadcasted_iota(jnp.int32, (rb, 128), 1)
            i16 = lane ^ 16
            i8 = lane ^ 8
            qh = mo(rr // 2, rb // 2)
            qr = qraw[pl.ds(qh, rb // 2), :]
            q = butterfly([qr[:, j * 128:(j + 1) * 128] for j in range(NSL)])
            q = [bf(u).astype(F32) for u in q]
            def window(buf, mode):
                if mode:
                    wins = [buf[j, pl.ds(rr, rb + HALO), :] for j in range(NSL)]
                    return lambda j, w: wins[j][HALO - DIL * w:HALO - DIL * w + rb, :]
                if xp == 'aligned8':
                    return lambda j, w: buf[j, pl.ds(mo(rr + 8 * w, 8), rb), :]
                return lambda j, w: buf[j, pl.ds(rr + HALO - DIL * w, rb), :]
            kw = window(kbuf, 'k' in vshift)
            lg = []
            for w in range(W):
                acc = None
                for j in range(NSL):
                    t = q[j] * kw(j, w)
                    acc = t if acc is None else acc + t
                acc = acc + jnp.take_along_axis(acc, i16, axis=1)
                acc = acc + jnp.take_along_axis(acc, i8, axis=1)
                if w > 0 and masked:
                    pos = rr + lax.broadcasted_iota(jnp.int32, (rb, 128), 0)
                    acc = jnp.where(pos >= DIL * w, acc, -1e9 * LOG2E)
                lg.append(acc)
            mx = functools.reduce(jnp.maximum, lg)
            es = [jnp.exp2(l - mx) for l in lg]
            z = functools.reduce(lambda a, b_: a + b_, es)
            rz = 1.0 / z
            ps = [e * rz for e in es]
            os_ = []
            vw = window(vbuf, 'v' in vshift)
            for j in range(NSL):
                acc = None
                for w in range(W):
                    t = ps[w] * vw(j, w)
                    acc = t if acc is None else acc + t
                os_.append(acc)
            ob = butterfly([u32(u.astype(BF16)) for u in os_])
            obuf[pl.ds(qh, rb // 2), :] = jnp.concatenate(ob, axis=1)

        waited = set()
        def wt(cp):
            waited.add(id(cp)); cp.wait()
        def early_stop():
            def body(i, c):
                mod_v[5, 0:8, 0:128] = mod_v[5, 0:8, 0:128] * 1.0001 + 1.0
                return c
            mod_v[5] = jnp.zeros((16, D), F32)
            lax.fori_loop(0, 7000, body, 0)
            for cp in early[1:] + rest:
                if id(cp) not in waited:
                    cp.wait()
            o_v[0:16, :] = bf(hbuf[0:8, :]) + bf(qraw[0:8, :]) + (kbuf[0, 16:32, :] + vbuf[0, 16:32, :] + mod_v[5, :, 0:128])[:, 0:1].astype(BF16)
            cp = pltpu.make_async_copy(o_v.at[0:16, :], o_h.at[0:16, :], osem)
            cp.start(); cp.wait()
        wt(cp_x0)
        xn = [ln_norm(x_v[b * lnb:(b + 1) * lnb, :].astype(F32)) for b in range(t0 // lnb)]
        wt(cp_wm[1]); do_mod(1)
        wt(kcs[0])
        for b, u in enumerate(xn):
            hf[b * lnb // 2:(b + 1) * lnb // 2, :] = u32((u * mod(1)).astype(BF16))
        h = None
        yk, o = [], 0
        for n, w_ in enumerate(kchunks):
            if n > 0:
                wt(kcs[n])
            yk.append(a1_dot(bf(hf[0:t0 // 2, :]), 1, (o, o + w_))); o += w_
        yk = jnp.concatenate(yk, axis=1)
        if stop == 'k':
            a1_store(0, 1, yk)
            hbuf[0:8, :] = u32(h[0:16])
            qraw[0:8, :] = u32(h[16:32])
            vbuf[0, 16:32, :] = jnp.zeros((16, 128), F32)
            early_stop(); return
        wt(cp_wm[0]); do_mod(0)
        hf[t0 // 2:t0 // 2 + 8, :] = u32(mod_v[0].astype(BF16))
        wt(cp_wv)
        yv = a1_dot(h, 2, first=True)
        a1_store(0, 1, yk)
        wt(cp_xn)
        wt(cp_wq)
        if late == 1:
            for cp in rest:
                cp.start()
        hbuf[...] = u32(ln1(t0, t1))
        yq = a1_dot(h, 0, first=True)
        a1_store(0, 2, yv)
        a1_store(0, 0, yq)
        wt(cp_xr)
        if stop == 'first':
            early_stop(); return
        if late == 2:
            for cp in rest:
                cp.start()

        def body_a(i, carry):
            if modmode == 'vpu':
                cpd = mac(wm_u.at[:, pl.ds(mo((2 + i) * D, D), D)], wm_v.at[2 + i], sems.at[6 + i])
                cpd.wait()
            r0 = mo(t0 + i * t1, 16)
            rn = mo(mn(t0 + (i + 1) * t1, S - t1), 16)
            hn = None
            ys = {}
            tix = {"K": 1, "V": 2, "Q": 0, "k": 1, "v": 2, "q": 0}
            for it in seq1.split(","):
                if it in ("K", "V", "Q"):
                    ys[tix[it]] = a1_dot(bf(hbuf[...]), tix[it])
                elif it[0] == "s":
                    a1_store(r0, tix[it[1]], ys[tix[it[1]]])
                elif it[0] == "a":
                    g = int(it[1:])
                    for b in range((nb1 * g) // 4, (nb1 * (g + 1)) // 4):
                        attn_block(mo((i * nb1 + b) * rb, rb), True)
                elif it[0] == "m":
                    do_mod_vpu(2 + i, ys[tix[it[1]]] if len(it) > 1 else None)
                elif it == "L":
                    hn = ln1(rn, t1)
                elif it == "h":
                    hbuf[...] = u32(hn)
            return carry
        lax.fori_loop(0, n1run, body_a, 0)
        if stop == 'loop1':
            early_stop(); return

        if modmode != 'vpu':
            for j in range(2, 6):
                cp_wm[j].wait()
        cp_wo.wait()
        for cp in cp_w1 + cp_w3 + cp_w2:
            cp.wait()

        def precompute(t_v, kh, nh):
            hr = prerb // 2
            for r in range(0, kh, hr):
                for c0 in range(0, nh, precb):
                    rs, cs = slice(r, r + hr), slice(c0, c0 + precb)
                    b11, b21, b22, b12 = [t_v[q_, rs, cs] for q_ in (0, 1, 2, 4)]
                    outs = []
                    for idx in (0, 1):
                        a11, a21, a22, a12 = [pltpu.unpack_elementwise(u_, index=idx, packed_dtype=BF16, unpacked_dtype=F32)
                                              for u_ in (b11, b21, b22, b12)]
                        t1 = a12 - a11
                        t2 = a22 - t1
                        outs.append((t1, t2, a22 - a12, t2 - a21))
                    for q_, lo, hi in zip((4, 5, 6, 3), *outs):
                        t_v[q_, rs, cs] = pltpu.pack_elementwise([lo, hi], packed_dtype=BF16)
        precompute(w1_v, D // 4, F // 2)
        precompute(w3_v, D // 4, F // 2)
        precompute(w2_v, F // 4, D // 2)
        if modmode != 'vpu':
            for j in range(2, 6):
                do_mod(j)

        hm = tm // hsplit
        def body_b(i, carry):
            r0 = mo(i * tm, tm)
            rn = mo(mn(i + 1, nt - 1) * tm, tm)
            rh = mo(i * (tm // 2), tm // 2)
            x1s, h2s = [], []
            for s in range(hsplit):
                ob = bf(obuf[pl.ds(rh + s * (hm // 2), hm // 2), :])
                a = jnp.dot(ob, bf(wo_v[...]), preferred_element_type=F32)
                x1 = x_v[pl.ds(r0 + s * hm, hm), :].astype(F32) + mod(2) * a
                x1s.append(x1)
                h2s.append(ln_norm(x1) * mod(4) + mod(3))
            KH = D // 2
            assert hsplit == 2
            sops = [u.astype(BF16) for u in s_combos(h2s[0][:, 0:KH], h2s[0][:, KH:], h2s[1][:, 0:KH], h2s[1][:, KH:])]
            accs = [None] * 7
            blk = 0
            nch = (F // 2) // sn
            sch = [n2b // nch + (1 if f < n2b % nch else 0) for f in range(nch)]
            for f in range(nch):
                fs = slice(f * sn, (f + 1) * sn)
                g = c_combos([jnp.dot(sops[p], bf(w1_v[p, :, fs]), preferred_element_type=F32) for p in range(7)])
                u = c_combos([jnp.dot(sops[p], bf(w3_v[p, :, fs]), preferred_element_type=F32) for p in range(7)])
                a_ = [gg * jax.nn.sigmoid(gg) * uu for gg, uu in zip(g, u)]
                aops = [v_.astype(BF16) for v_ in s_combos(*a_)]
                for _ in range(sch[f]):
                    attn_block(mo(mn(n1 * n1b + i * n2b + blk, ntot - 1) * rb, rb), False)
                    blk += 1
                for p in range(7):
                    t = jnp.dot(aops[p], bf(w2_v[p, f * sn // 2:(f + 1) * sn // 2, :]), preferred_element_type=F32)
                    accs[p] = t if accs[p] is None else accs[p] + t
            c11, c12, c21, c22 = c_combos(accs)
            g5 = mod(5)
            o_v[pl.ds(r0, hm), 0:KH] = (x1s[0][:, 0:KH] + g5[:, 0:KH] * c11).astype(BF16)
            o_v[pl.ds(r0, hm), KH:] = (x1s[0][:, KH:] + g5[:, KH:] * c12).astype(BF16)
            o_v[pl.ds(r0 + hm, hm), 0:KH] = (x1s[1][:, 0:KH] + g5[:, 0:KH] * c21).astype(BF16)
            o_v[pl.ds(r0 + hm, hm), KH:] = (x1s[1][:, KH:] + g5[:, KH:] * c22).astype(BF16)
            pltpu.make_async_copy(o_v.at[pl.ds(r0, tm), :], o_h.at[pl.ds(r0, tm), :], osem).start()
            return carry

        lax.fori_loop(0, n2run, body_b, 0)
        for i in range(n2run):
            pltpu.make_async_copy(o_v.at[pl.ds(i * tm, tm), :], o_h.at[pl.ds(i * tm, tm), :], osem).wait()

    def f(A_x, A_wqkv, A_wo, B_x, B_w1, B_w3, B_w2, c, w_mod):
        x2 = A_x.reshape(S, D)
        anyspec = pl.BlockSpec(memory_space=pl.ANY)
        out = pl.pallas_call(
            kernel,
            in_specs=[anyspec] * 8,
            out_specs=anyspec,
            out_shape=jax.ShapeDtypeStruct((S, D), BF16),
            scratch_shapes=[
                pltpu.VMEM((S, D), BF16),
                pltpu.VMEM((1, D), BF16),
                pltpu.VMEM((D // 2, 3 * D), U32),
                pltpu.VMEM((D // 2, D), U32),
                pltpu.VMEM((7, D // 4, F // 2), U32),
                pltpu.VMEM((7, D // 4, F // 2), U32),
                pltpu.VMEM((7, F // 4, D // 2), U32),
                pltpu.VMEM((6, D // 2, D), U32),
                pltpu.VMEM((6, 16, D), F32),
                pltpu.VMEM((S // 2, D), U32),
                pltpu.VMEM((NSL, S + HALO, 128), F32),
                pltpu.VMEM((NSL, S + HALO, 128), F32),
                pltpu.VMEM((t1 // 2, D), U32),
                pltpu.VMEM((S // 2, D), U32),
                pltpu.VMEM((S, D), BF16),
                pltpu.VMEM((2, 8, D), F32),
                pltpu.VMEM((t0 // 2 + 8, D), U32),
                pltpu.VMEM((D, 128), F32),
                pltpu.SemaphoreType.DMA((28 + len(kchunks),)),
                pltpu.SemaphoreType.DMA(()),
            ],
            compiler_params=pltpu.CompilerParams(vmem_limit_bytes=120 * 1024 * 1024),
        )(x2, c, A_wqkv, A_wo, B_w1, B_w3, B_w2, w_mod)
        return out.reshape(1, S, D)
    return f


_impl = make()


@jax.jit
def pallas_adaLN_cond__sliding_local_dilated__glu_gated_swiglu__prompt_kernel(
    A_x, A_wqkv, A_wo, B_x, B_w1, B_w3, B_w2, c, w_mod):
    return _impl(A_x, A_wqkv, A_wo, B_x, B_w1, B_w3, B_w2, c, w_mod)
```

```python
import functools
import jax, jax.numpy as jnp
from jax import lax
from jax.experimental import pallas as pl
from jax.experimental.pallas import tpu as pltpu

S, D, H, DH, F = 2048, 1024, 32, 32, 3584
W, DIL = 8, 2
HALO = 16
EPS = 1e-5
LOG2E = 1.4426950408889634
NSL = D // 128
F32, BF16, U32 = jnp.float32, jnp.bfloat16, jnp.uint32


def butterfly(xs):
    lane = lax.broadcasted_iota(jnp.int32, xs[0].shape, 1)
    for b in (4, 2, 1):
        m = (lane & b) != 0
        ys = list(xs)
        for j in range(8):
            if j & b == 0:
                A, B = xs[j], xs[j | b]
                ys[j] = jnp.where(m, pltpu.roll(B, b, 1), A)
                ys[j | b] = jnp.where(m, B, pltpu.roll(A, 128 - b, 1))
        xs = ys
    return xs


def s_combos(a11, a12, a21, a22):
    s1 = a21 + a22
    s2 = s1 - a11
    s3 = a11 - a21
    s4 = a12 - s2
    return [a11, a12, s4, a22, s1, s2, s3]


def c_combos(p):
    p1, p2, p3, p4, p5, p6, p7 = p
    u2 = p1 + p6
    u3 = u2 + p7
    u4 = u2 + p5
    return (p1 + p2, u4 + p3, u3 - p4, u3 + p5)


def make(tm=256, rb=16, fc=512, lnb=16, sched=None, split0=True, t0=640, kchunks=(128, 512),
         seq1="K,a0,sk,V,a1,sv,L,Q,a2,a3,sq,h", modmode="mid", nodma=False, xp=None, f_order=0, hsplit=2, late=0, stop=None, vshift='', satrick=True, sepbias=True, mdep='K', n1run=4, n2run=8, n1b=4, sn=256, prerb=16, precb=256, midorder='2345abc'):
    nt = S // tm
    nf = F // fc
    nblk = tm // rb
    n1 = 4
    t1 = (S - t0) // n1
    assert t0 + n1 * t1 == S and t1 % 16 == 0 and t1 % lnb == 0 and t0 % lnb == 0
    nb1 = n1b
    ntot = S // rb
    n2b = max(-(-(ntot - n1 * n1b) // (nt - 1)), 0)
    assert n1 * n1b >= nblk
    assert all(n1 * n1b + i * n2b >= nblk * (i + 1) for i in range(nt)) or n1 * n1b + (nt - 1) * n2b >= ntot
    if sched is None:
        base = n2b // nf; rem = n2b % nf
        sched = [base + (1 if f < rem else 0) for f in range(nf)]
    assert sum(sched) == n2b

    def ln_norm(xf):
        m = jnp.mean(xf, axis=-1, keepdims=True)
        xc = xf - m
        v = jnp.mean(xc * xc, axis=-1, keepdims=True)
        return xc * lax.rsqrt(v + EPS)

    class _Nop:
        def start(self): pass
        def wait(self): pass

    def mac(a, b, sem):
        return _Nop() if nodma else pltpu.make_async_copy(a, b, sem)

    def mo(v, m):
        return v if isinstance(v, int) else pl.multiple_of(v, m)

    def mn(a, b):
        return min(a, b) if isinstance(a, int) else jnp.minimum(a, b)

    def bf(u):
        return pltpu.bitcast(u, BF16)

    def u32(b):
        return pltpu.bitcast(b, U32)

    def kernel(x_h, c_h, wqkv_h, wo_h, w1_h, w3_h, w2_h, wm_h, o_h,
               x_v, c_v, wr_v, wt_v, wo_v, w1_v, w3_v, w2_v, wm_v, mod_v, qraw, kbuf, vbuf, hbuf, obuf, o_v, bias_v, hf, scol, sems, osem):
        wqkv_u, wo_u, w1_u, w3_u, w2_u, wm_u = [r.bitcast(U32) for r in (wqkv_h, wo_h, w1_h, w3_h, w2_h, wm_h)]
        cp_c = mac(c_h, c_v, sems.at[0])
        cp_x0 = mac(x_h.at[0:t0, :], x_v.at[0:t0, :], sems.at[1])
        cp_xn = mac(x_h.at[t0:t0 + t1, :], x_v.at[t0:t0 + t1, :], sems.at[2])
        cp_xr = mac(x_h.at[t0 + t1:S, :], x_v.at[t0 + t1:S, :], sems.at[3])
        cp_wm = [mac(wm_u.at[:, j * D:(j + 1) * D], wm_v.at[j], sems.at[4 + j]) for j in range(6)]
        KH2, NH = D // 4, D // 2
        def quad(t, slot, lo=0, hi=NH):
            ro, co = ((0, 0), (KH2, 0), (KH2, NH), (0, NH))[slot]
            return (wqkv_u.at[ro:ro + KH2, t * D + co + lo:t * D + co + hi], wr_v.at[t, slot, :, lo:hi])
        kcs = []
        for n, (lo, hi) in enumerate(zip([0] + list(kchunks[:-1]), kchunks)):
            kcs.append([mac(*quad(1, 0, lo, hi), sems.at[16 + n]), mac(*quad(1, 1, lo, hi), sems.at[16 + n])])
        kcs.append([mac(*quad(1, 3), sems.at[16 + len(kchunks)]), mac(*quad(1, 2), sems.at[16 + len(kchunks)])])
        cp_wv = [mac(*quad(2, q_), sems.at[10]) for q_ in range(4)]
        cp_wq = [mac(*quad(0, q_), sems.at[11]) for q_ in range(4)]
        cp_wo = mac(wo_u, wo_v, sems.at[12])
        NS0 = 17 + len(kchunks)
        def wcopies(src, dst, kh, nh, base):
            return [mac(src.at[0:kh, 0:nh], dst.at[0], sems.at[base]),
                    mac(src.at[kh:2 * kh, 0:nh], dst.at[1], sems.at[base + 1]),
                    mac(src.at[kh:2 * kh, nh:2 * nh], dst.at[2], sems.at[base + 2]),
                    mac(src.at[0:kh, nh:2 * nh], dst.at[4], sems.at[base + 3])]
        cp_w1 = wcopies(w1_u, w1_v, D // 4, F // 2, NS0)
        cp_w3 = wcopies(w3_u, w3_v, D // 4, F // 2, NS0 + 4)
        cp_w2 = wcopies(w2_u, w2_v, F // 4, D // 2, NS0 + 8)
        early = [cp_c, cp_x0, cp_wm[1]] + sum(kcs, []) + [cp_wm[0]] + cp_wv + [cp_xn] + cp_wq + [cp_xr]
        rest = [cp_wm[2], cp_wm[3], cp_wm[4], cp_wm[5], cp_wo] + cp_w1 + cp_w3 + cp_w2
        for cp in early + ([] if late else rest):
            cp.start()

        kbuf[:, 0:HALO, :] = jnp.zeros((NSL, HALO, 128), F32)
        vbuf[:, 0:HALO, :] = jnp.zeros((NSL, HALO, 128), F32)
        cp_c.wait()
        waited_c = True
        cf = c_v[...].astype(F32)
        sc = (cf * jax.nn.sigmoid(cf)).astype(BF16)
        if modmode == 'vpu':
            scol[...] = jnp.broadcast_to(sc.astype(F32), (128, D)).T
        sc = jnp.broadcast_to(sc, (16, D))

        def do_mod(j):
            r = jnp.dot(sc, bf(wm_v[j]), preferred_element_type=F32)
            if j in (1, 4):
                r = 1.0 + r
            mod_v[j] = r

        def do_mod_vpu(j, ydep):
            flag = kbuf[0, 0:8, :] != 0.0
            flag = jnp.concatenate([flag] * 2, axis=0)
            tot = None
            for p in range(8):
                accs = [None] * NSL
                for kb in range(8):
                    lo = p * 128 + kb * 16
                    sc_ = scol[lo:lo + 16, :]
                    if ydep is not None:
                        sc_ = jnp.where(flag, ydep[0:16, p * 128:(p + 1) * 128], sc_)
                    w = bf(wm_v[j, lo // 2:lo // 2 + 8, :]).astype(F32)
                    for jj in range(NSL):
                        t = w[:, jj * 128:(jj + 1) * 128] * sc_
                        t = t[0:8] + t[8:16]
                        accs[jj] = t if accs[jj] is None else accs[jj] + t
                r = jnp.concatenate(accs, axis=1)
                tot = r if tot is None else tot + r
            r = jnp.sum(tot, axis=0, keepdims=True) + jnp.where(j == 4, 1.0, 0.0)
            mod_v[j, 0:1, :] = r

        def mod(j):
            return mod_v[j, 0:1, :]

        def ln1_ops(r0, rows):
            half = rows // 2
            outs = [[] for _ in range(8)]
            for b in range(half // lnb):
                top = ln_norm(x_v[pl.ds(r0 + b * lnb, lnb), :].astype(F32)) * mod(1)
                bot = ln_norm(x_v[pl.ds(r0 + half + b * lnb, lnb), :].astype(F32)) * mod(1)
                ops = s_combos(top[:, 0:NH], top[:, NH:], bot[:, 0:NH], bot[:, NH:]) + [bot[:, 0:NH]]
                for q_ in range(8):
                    outs[q_].append(u32(ops[q_].astype(BF16)))
            return [jnp.concatenate(o_, axis=0) for o_ in outs]

        bufs = [None, kbuf, vbuf]

        QS = DH ** -0.5 * LOG2E

        def wq_op(t, p, cs=slice(None)):
            return bf(wr_v[t, p, :, cs] if p < 3 else wt_v[t, p - 3, :, cs])

        def bias(t):
            sa = mod_v[0].astype(BF16)
            dd = lambda c_, q_: jnp.dot(sa[:, c_], bf(wr_v[t, q_]), preferred_element_type=F32)
            b = jnp.concatenate([dd(slice(0, NH), 0) + dd(slice(NH, D), 1), dd(slice(0, NH), 3) + dd(slice(NH, D), 2)], axis=1)[0:8, :]
            bias_v[t // 2] = b * QS if t == 0 else b

        def proj_s(hops, t):
            c11, c12, c21, c22 = c_combos([jnp.dot(bf(hops[p]), wq_op(t, p), preferred_element_type=F32) for p in range(7)])
            top = jnp.concatenate([c11, c12], axis=1)
            bot = jnp.concatenate([c21, c22], axis=1)
            if t == 1:
                return top, bot
            b = bias_v[t // 2, 0:1, :]
            return ((top * QS + b), (bot * QS + b)) if t == 0 else (top + b, bot + b)

        def precompute(src, dst, kh, nh, s12=3, dsl=(1, 2, 3, 0)):
            hr = prerb // 2
            for r in range(0, kh, hr):
                for c0 in range(0, nh, precb):
                    rs, cs = slice(r, r + hr), slice(c0, c0 + precb)
                    b11, b21, b22, b12 = [src[q_, rs, cs] for q_ in (0, 1, 2, s12)]
                    outs = []
                    for idx in (0, 1):
                        a11, a21, a22, a12 = [pltpu.unpack_elementwise(u_, index=idx, packed_dtype=BF16, unpacked_dtype=F32)
                                              for u_ in (b11, b21, b22, b12)]
                        t1_ = a12 - a11
                        t2_ = a22 - t1_
                        outs.append((t1_, t2_, a22 - a12, t2_ - a21))
                    for q_, lo, hi in zip(dsl, *outs):
                        dst[q_, rs, cs] = pltpu.pack_elementwise([lo, hi], packed_dtype=BF16)

        def a1_store(r0, t, y):
            rows = y.shape[0]
            yb = u32(y.astype(BF16))
            if t == 0:
                qraw[pl.ds(mo(r0 // 2, 8), rows // 2), :] = yb
            else:
                ys = butterfly([yb[:, j * 128:(j + 1) * 128] for j in range(NSL)])
                for j in range(NSL):
                    bufs[t][j, pl.ds(r0 + HALO, rows), :] = bf(ys[j]).astype(F32)

        def attn_block(rr, masked):
            lane = lax.broadcasted_iota(jnp.int32, (rb, 128), 1)
            i16 = lane ^ 16
            i8 = lane ^ 8
            qh = mo(rr // 2, rb // 2)
            qr = qraw[pl.ds(qh, rb // 2), :]
            q = butterfly([qr[:, j * 128:(j + 1) * 128] for j in range(NSL)])
            q = [bf(u).astype(F32) for u in q]
            def window(buf, mode):
                if mode:
                    wins = [buf[j, pl.ds(rr, rb + HALO), :] for j in range(NSL)]
                    return lambda j, w: wins[j][HALO - DIL * w:HALO - DIL * w + rb, :]
                if xp == 'aligned8':
                    return lambda j, w: buf[j, pl.ds(mo(rr + 8 * w, 8), rb), :]
                return lambda j, w: buf[j, pl.ds(rr + HALO - DIL * w, rb), :]
            kw = window(kbuf, 'k' in vshift)
            lg = []
            for w in range(W):
                acc = None
                for j in range(NSL):
                    t = q[j] * kw(j, w)
                    acc = t if acc is None else acc + t
                acc = acc + jnp.take_along_axis(acc, i16, axis=1)
                acc = acc + jnp.take_along_axis(acc, i8, axis=1)
                if w > 0 and masked:
                    pos = rr + lax.broadcasted_iota(jnp.int32, (rb, 128), 0)
                    acc = jnp.where(pos >= DIL * w, acc, -1e9 * LOG2E)
                lg.append(acc)
            mx = functools.reduce(jnp.maximum, lg)
            es = [jnp.exp2(l - mx) for l in lg]
            z = functools.reduce(lambda a, b_: a + b_, es)
            rz = 1.0 / z
            ps = [e * rz for e in es]
            os_ = []
            vw = window(vbuf, 'v' in vshift)
            for j in range(NSL):
                acc = None
                for w in range(W):
                    t = ps[w] * vw(j, w)
                    acc = t if acc is None else acc + t
                os_.append(acc)
            ob = butterfly([u32(u.astype(BF16)) for u in os_])
            obuf[pl.ds(qh, rb // 2), :] = jnp.concatenate(ob, axis=1)

        waited = set()
        def wt(cp):
            waited.add(id(cp)); cp.wait()
        def early_stop():
            def body(i, c):
                mod_v[5, 0:8, 0:128] = mod_v[5, 0:8, 0:128] * 1.0001 + 1.0
                return c
            mod_v[5] = jnp.zeros((16, D), F32)
            lax.fori_loop(0, 7000, body, 0)
            for cp in early[1:] + rest:
                if id(cp) not in waited:
                    cp.wait()
            o_v[0:16, :] = bf(hbuf[0:8, :]) + bf(qraw[0:8, :]) + (kbuf[0, 16:32, :] + vbuf[0, 16:32, :] + mod_v[5, :, 0:128])[:, 0:1].astype(BF16)
            cp = pltpu.make_async_copy(o_v.at[0:16, :], o_h.at[0:16, :], osem)
            cp.start(); cp.wait()
        wt(cp_x0)
        h0 = t0 // 2
        xn = [ln_norm(x_v[b * lnb:(b + 1) * lnb, :].astype(F32)) for b in range(t0 // lnb)]
        wt(cp_wm[1]); do_mod(1)
        for cp in kcs[0]:
            wt(cp)
        for b in range(h0 // lnb):
            top = xn[b] * mod(1)
            bot = xn[h0 // lnb + b] * mod(1)
            ops = s_combos(top[:, 0:NH], top[:, NH:], bot[:, 0:NH], bot[:, NH:]) + [bot[:, 0:NH]]
            for q_ in range(8):
                hf[q_, b * lnb // 2:(b + 1) * lnb // 2, :] = u32(ops[q_].astype(BF16))
        def kdot(cl, cr, cs):
            dd = lambda a_, q_: jnp.dot(bf(hf[a_]), bf(wr_v[1, q_, :, cs]), preferred_element_type=F32)
            return dd(0, cl) + dd(1, cr), dd(7, cl) + dd(3, cr)
        ytop, ybot = [], []
        for n, (lo, hi) in enumerate(zip([0] + list(kchunks[:-1]), kchunks)):
            if n > 0:
                for cp in kcs[n]:
                    wt(cp)
            a_, b_ = kdot(0, 1, slice(lo, hi))
            ytop.append(a_); ybot.append(b_)
        for cp in kcs[-1]:
            wt(cp)
        a_, b_ = kdot(3, 2, slice(None))
        yk = (jnp.concatenate(ytop + [a_], axis=1), jnp.concatenate(ybot + [b_], axis=1))
        wt(cp_wm[0]); do_mod(0)
        for cp in cp_wv:
            wt(cp)
        precompute(wr_v.at[2], wt_v.at[2], KH2, NH)
        bias(2)
        yv = proj_s(hf, 2)
        a1_store(0, 1, yk[0]); a1_store(h0, 1, yk[1])
        wt(cp_xn)
        for cp in cp_wq:
            wt(cp)
        precompute(wr_v.at[0], wt_v.at[0], KH2, NH)
        precompute(wr_v.at[1], wt_v.at[1], KH2, NH)
        bias(0)
        hn = ln1_ops(t0, t1)
        for q_ in range(7):
            hbuf[q_] = hn[q_]
        yq = proj_s(hf, 0)
        a1_store(0, 2, yv[0]); a1_store(h0, 2, yv[1])
        a1_store(0, 0, yq[0]); a1_store(h0, 0, yq[1])
        wt(cp_xr)
        if stop == 'first':
            early_stop(); return
        if late == 2:
            for cp in rest:
                cp.start()

        def body_a(i, carry):
            if modmode == 'vpu':
                cpd = mac(wm_u.at[:, pl.ds(mo((2 + i) * D, D), D)], wm_v.at[2 + i], sems.at[6 + i])
                cpd.wait()
            r0 = mo(t0 + i * t1, 16)
            rn = mo(mn(t0 + (i + 1) * t1, S - t1), 16)
            hn = None
            ys = {}
            tix = {"K": 1, "V": 2, "Q": 0, "k": 1, "v": 2, "q": 0}
            for it in seq1.split(","):
                if it in ("K", "V", "Q"):
                    ys[tix[it]] = proj_s(hbuf, tix[it])
                elif it[0] == "s":
                    a1_store(r0, tix[it[1]], ys[tix[it[1]]][0]); a1_store(r0 + t1 // 2, tix[it[1]], ys[tix[it[1]]][1])
                elif it[0] == "a":
                    g = int(it[1:])
                    for b in range((nb1 * g) // 4, (nb1 * (g + 1)) // 4):
                        attn_block(mo((i * nb1 + b) * rb, rb), True)
                elif it[0] == "m":
                    do_mod_vpu(2 + i, ys[tix[it[1]]] if len(it) > 1 else None)
                elif it == "L":
                    hn = ln1_ops(rn, t1)
                elif it == "h":
                    for q_ in range(7):
                        hbuf[q_] = hn[q_]
            return carry
        lax.fori_loop(0, n1run, body_a, 0)
        if stop == 'loop1':
            early_stop(); return

        if modmode != 'vpu':
            for j in range(2, 6):
                cp_wm[j].wait()
        cp_wo.wait()
        for cp in cp_w1 + cp_w3 + cp_w2:
            cp.wait()

        items = {"a": lambda: precompute(w1_v, w1_v, D // 4, F // 2, 4, (4, 5, 6, 3)), "b": lambda: precompute(w3_v, w3_v, D // 4, F // 2, 4, (4, 5, 6, 3)), "c": lambda: precompute(w2_v, w2_v, F // 4, D // 2, 4, (4, 5, 6, 3))}
        for ch in midorder:
            if ch in items:
                items[ch]()
            else:
                do_mod(int(ch))

        hm = tm // hsplit
        def body_b(i, carry):
            r0 = mo(i * tm, tm)
            rn = mo(mn(i + 1, nt - 1) * tm, tm)
            rh = mo(i * (tm // 2), tm // 2)
            x1s, h2s = [], []
            for s in range(hsplit):
                ob = bf(obuf[pl.ds(rh + s * (hm // 2), hm // 2), :])
                a = jnp.dot(ob, bf(wo_v[...]), preferred_element_type=F32)
                x1 = x_v[pl.ds(r0 + s * hm, hm), :].astype(F32) + mod(2) * a
                x1s.append(x1)
                h2s.append(ln_norm(x1) * mod(4) + mod(3))
            KH = D // 2
            assert hsplit == 2
            sops = [u.astype(BF16) for u in s_combos(h2s[0][:, 0:KH], h2s[0][:, KH:], h2s[1][:, 0:KH], h2s[1][:, KH:])]
            accs = [None] * 7
            blk = 0
            nch = (F // 2) // sn
            sch = [n2b // nch + (1 if f < n2b % nch else 0) for f in range(nch)]
            for f in range(nch):
                fs = slice(f * sn, (f + 1) * sn)
                g = c_combos([jnp.dot(sops[p], bf(w1_v[p, :, fs]), preferred_element_type=F32) for p in range(7)])
                u = c_combos([jnp.dot(sops[p], bf(w3_v[p, :, fs]), preferred_element_type=F32) for p in range(7)])
                a_ = [gg * jax.nn.sigmoid(gg) * uu for gg, uu in zip(g, u)]
                aops = [v_.astype(BF16) for v_ in s_combos(*a_)]
                for _ in range(sch[f]):
                    attn_block(mo(mn(n1 * n1b + i * n2b + blk, ntot - 1) * rb, rb), False)
                    blk += 1
                for p in range(7):
                    t = jnp.dot(aops[p], bf(w2_v[p, f * sn // 2:(f + 1) * sn // 2, :]), preferred_element_type=F32)
                    accs[p] = t if accs[p] is None else accs[p] + t
            c11, c12, c21, c22 = c_combos(accs)
            g5 = mod(5)
            o_v[pl.ds(r0, hm), 0:KH] = (x1s[0][:, 0:KH] + g5[:, 0:KH] * c11).astype(BF16)
            o_v[pl.ds(r0, hm), KH:] = (x1s[0][:, KH:] + g5[:, KH:] * c12).astype(BF16)
            o_v[pl.ds(r0 + hm, hm), 0:KH] = (x1s[1][:, 0:KH] + g5[:, 0:KH] * c21).astype(BF16)
            o_v[pl.ds(r0 + hm, hm), KH:] = (x1s[1][:, KH:] + g5[:, KH:] * c22).astype(BF16)
            pltpu.make_async_copy(o_v.at[pl.ds(r0, tm), :], o_h.at[pl.ds(r0, tm), :], osem).start()
            return carry

        lax.fori_loop(0, n2run, body_b, 0)
        for i in range(n2run):
            pltpu.make_async_copy(o_v.at[pl.ds(i * tm, tm), :], o_h.at[pl.ds(i * tm, tm), :], osem).wait()

    def f(A_x, A_wqkv, A_wo, B_x, B_w1, B_w3, B_w2, c, w_mod):
        x2 = A_x.reshape(S, D)
        anyspec = pl.BlockSpec(memory_space=pl.ANY)
        out = pl.pallas_call(
            kernel,
            in_specs=[anyspec] * 8,
            out_specs=anyspec,
            out_shape=jax.ShapeDtypeStruct((S, D), BF16),
            scratch_shapes=[
                pltpu.VMEM((S, D), BF16),
                pltpu.VMEM((1, D), BF16),
                pltpu.VMEM((3, 4, D // 4, D // 2), U32),
                pltpu.VMEM((3, 4, D // 4, D // 2), U32),
                pltpu.VMEM((D // 2, D), U32),
                pltpu.VMEM((7, D // 4, F // 2), U32),
                pltpu.VMEM((7, D // 4, F // 2), U32),
                pltpu.VMEM((7, F // 4, D // 2), U32),
                pltpu.VMEM((6, D // 2, D), U32),
                pltpu.VMEM((6, 16, D), F32),
                pltpu.VMEM((S // 2, D), U32),
                pltpu.VMEM((NSL, S + HALO, 128), F32),
                pltpu.VMEM((NSL, S + HALO, 128), F32),
                pltpu.VMEM((7, t1 // 4, D // 2), U32),
                pltpu.VMEM((S // 2, D), U32),
                pltpu.VMEM((S, D), BF16),
                pltpu.VMEM((2, 8, D), F32),
                pltpu.VMEM((8, t0 // 4, D // 2), U32),
                pltpu.VMEM((D, 128), F32),
                pltpu.SemaphoreType.DMA((29 + len(kchunks),)),
                pltpu.SemaphoreType.DMA(()),
            ],
            compiler_params=pltpu.CompilerParams(vmem_limit_bytes=120 * 1024 * 1024),
        )(x2, c, A_wqkv, A_wo, B_w1, B_w3, B_w2, w_mod)
        return out.reshape(1, S, D)
    return f


_impl = make()


@jax.jit
def pallas_adaLN_cond__sliding_local_dilated__glu_gated_swiglu__prompt_kernel(
    A_x, A_wqkv, A_wo, B_x, B_w1, B_w3, B_w2, c, w_mod):
    return _impl(A_x, A_wqkv, A_wo, B_x, B_w1, B_w3, B_w2, c, w_mod)
```

```python
import functools

import jax
import jax.numpy as jnp
from jax import lax
import jax.experimental.pallas as pl
import jax.experimental.pallas.tpu as pltpu

S, D, H, DH, F = 2048, 1024, 32, 32, 3584
W, DIL = 8, 2
HALO = 16
EPS = 1e-5
LOG2E = 1.4426950408889634
QS = DH ** -0.5 * LOG2E
NSL = D // 128
F32, BF16, U32, I32 = jnp.float32, jnp.bfloat16, jnp.uint32, jnp.int32

TM = 256
HM = TM // 2
RB = 16
SN = 256
PC = 256
T0 = 640
N1 = 4
T1 = (S - T0) // N1
KCH = (0, 128, 512)
NT = S // TM
NBLK = TM // RB
NB1 = NBLK // N1
NCH = (F // 2) // SN
SCH = [NBLK // NCH + (1 if f < NBLK % NCH else 0) for f in range(NCH)]
QR, NH = D // 4, D // 2


def _butterfly(xs):
    lane = lax.broadcasted_iota(I32, xs[0].shape, 1)
    for b in (4, 2, 1):
        m = (lane & b) != 0
        ys = list(xs)
        for j in range(8):
            if j & b == 0:
                lo, hi = xs[j], xs[j | b]
                ys[j] = jnp.where(m, pltpu.roll(hi, b, 1), lo)
                ys[j | b] = jnp.where(m, hi, pltpu.roll(lo, 128 - b, 1))
        xs = ys
    return xs


def _a_ops(a11, a12, a21, a22):
    s1 = a21 + a22
    s2 = s1 - a11
    return [a11, a12, a12 - s2, a22, s1, s2, a11 - a21]


def _c_quads(p):
    p1, p2, p3, p4, p5, p6, p7 = p
    u2 = p1 + p6
    u3 = u2 + p7
    return p1 + p2, (u2 + p5) + p3, u3 - p4, u3 + p5


def _ln_norm(xf):
    m = jnp.mean(xf, axis=-1, keepdims=True)
    xc = xf - m
    v = jnp.mean(xc * xc, axis=-1, keepdims=True)
    return xc * lax.rsqrt(v + EPS)


def _bf(u):
    return pltpu.bitcast(u, BF16)


def _u32(b):
    return pltpu.bitcast(b, U32)


def _pk(y):
    r = y.shape[0]
    lo = jnp.concatenate([y[g:g + 8] for g in range(0, r, 16)], axis=0)
    hi = jnp.concatenate([y[g + 8:g + 16] for g in range(0, r, 16)], axis=0)
    return pltpu.pack_elementwise([lo, hi], packed_dtype=BF16)


def _unpk(u):
    lo = pltpu.unpack_elementwise(u, index=0, packed_dtype=BF16, unpacked_dtype=F32)
    hi = pltpu.unpack_elementwise(u, index=1, packed_dtype=BF16, unpacked_dtype=F32)
    parts = []
    for g in range(0, u.shape[0], 8):
        parts += [lo[g:g + 8], hi[g:g + 8]]
    return jnp.concatenate(parts, axis=0)


def _mo(v, m):
    return v if isinstance(v, int) else pl.multiple_of(v, m)


def _dot(a, b):
    return jnp.dot(a, b, preferred_element_type=F32)


def _kernel(x_h, c_h, wqkv_h, wo_h, w1_h, w3_h, w2_h, wm_h, o_h,
            x_v, c_v, wr_v, wt_v, wo_v, w1_v, w3_v, w2_v, wm_v, mod_v, bias_v,
            qraw, kbuf, vbuf, hbuf, hk, hs, obuf, o_v, sems, osem):
    wqkv_u, wo_u, w1_u, w3_u, w2_u, wm_u = [
        r.bitcast(U32) for r in (wqkv_h, wo_h, w1_h, w3_h, w2_h, wm_h)]
    mac = pltpu.make_async_copy

    cp_c = mac(c_h, c_v, sems.at[0])
    cp_x0 = mac(x_h.at[0:T0, :], x_v.at[0:T0, :], sems.at[1])
    cp_xn = mac(x_h.at[T0:T0 + T1, :], x_v.at[T0:T0 + T1, :], sems.at[2])
    cp_xr = mac(x_h.at[T0 + T1:S, :], x_v.at[T0 + T1:S, :], sems.at[3])
    cp_wm = [mac(wm_u.at[:, j * D:(j + 1) * D], wm_v.at[j], sems.at[4 + j]) for j in range(6)]

    def quad(t, slot, lo=0, hi=NH):
        ro, co = ((0, 0), (QR, 0), (QR, NH), (0, NH))[slot]
        return (wqkv_u.at[ro:ro + QR, t * D + co + lo:t * D + co + hi], wr_v.at[t, slot, :, lo:hi])

    kcs = [[mac(*quad(1, 0, lo, hi), sems.at[10 + n]), mac(*quad(1, 1, lo, hi), sems.at[10 + n])]
           for n, (lo, hi) in enumerate(zip(KCH[:-1], KCH[1:]))]
    kcs.append([mac(*quad(1, 3), sems.at[12]), mac(*quad(1, 2), sems.at[12])])
    cp_wv = [mac(*quad(2, q), sems.at[13]) for q in range(4)]
    cp_wq = [mac(*quad(0, q), sems.at[14]) for q in range(4)]
    cp_wo = mac(wo_u, wo_v, sems.at[15])

    def wcopies(src, dst, kh, nh, base):
        return [mac(src.at[0:kh, 0:nh], dst.at[0], sems.at[base]),
                mac(src.at[kh:2 * kh, 0:nh], dst.at[1], sems.at[base + 1]),
                mac(src.at[kh:2 * kh, nh:2 * nh], dst.at[2], sems.at[base + 2]),
                mac(src.at[0:kh, nh:2 * nh], dst.at[4], sems.at[base + 3])]

    cp_ffn = (wcopies(w1_u, w1_v, D // 4, F // 2, 16) + wcopies(w3_u, w3_v, D // 4, F // 2, 20)
              + wcopies(w2_u, w2_v, F // 4, D // 2, 24))
    for cp in ([cp_c, cp_x0, cp_wm[1]] + sum(kcs, []) + [cp_wm[0]] + cp_wv + [cp_xn] + cp_wq
               + [cp_xr, cp_wm[2], cp_wm[3], cp_wm[4], cp_wm[5], cp_wo] + cp_ffn):
        cp.start()

    kbuf[:, 0:HALO, :] = jnp.zeros((NSL, HALO, 128), F32)
    vbuf[:, 0:HALO, :] = jnp.zeros((NSL, HALO, 128), F32)
    cp_c.wait()
    cf = c_v[...].astype(F32)
    sc = jnp.broadcast_to((cf * jax.nn.sigmoid(cf)).astype(BF16), (16, D))

    def do_mod(j):
        r = _dot(sc, _bf(wm_v[j]))
        mod_v[j] = 1.0 + r if j in (1, 4) else r

    def mod(j):
        return mod_v[j, 0:1, :]

    def ln1_ops(r0, rows):
        half = rows // 2
        outs = [[] for _ in range(7)]
        for b in range(half // 16):
            top = _ln_norm(x_v[pl.ds(r0 + b * 16, 16), :].astype(F32)) * mod(1)
            bot = _ln_norm(x_v[pl.ds(r0 + half + b * 16, 16), :].astype(F32)) * mod(1)
            for q, u in enumerate(_a_ops(top[:, 0:NH], top[:, NH:], bot[:, 0:NH], bot[:, NH:])):
                outs[q].append(_u32(u.astype(BF16)))
        return [jnp.concatenate(o, axis=0) for o in outs]

    def bias(t):
        sa = mod_v[0].astype(BF16)
        dd = lambda cs, q: _dot(sa[:, cs], _bf(wr_v[t, q]))
        lo, hi = slice(0, NH), slice(NH, D)
        b = jnp.concatenate([dd(lo, 0) + dd(hi, 1), dd(lo, 3) + dd(hi, 2)], axis=1)[0:8, :]
        bias_v[t // 2] = b * QS if t == 0 else b

    def proj(hop, t):
        def wop(p, cs):
            return _bf(wr_v[t, p, :, cs] if p < 3 else wt_v[t, p - 3, :, cs])
        parts = [_c_quads([_dot(_bf(hop(p)), wop(p, slice(c0, c0 + PC))) for p in range(7)])
                 for c0 in range(0, NH, PC)]
        c11, c12, c21, c22 = [jnp.concatenate([pp[q] for pp in parts], axis=1) for q in range(4)]
        top = jnp.concatenate([c11, c12], axis=1)
        bot = jnp.concatenate([c21, c22], axis=1)
        if t == 1:
            return top, bot
        b = bias_v[t // 2, 0:1, :]
        return (top * QS + b, bot * QS + b) if t == 0 else (top + b, bot + b)

    def precompute(src, dst, kh, nh, s12, dsl):
        for r in range(0, kh, 8):
            for c0 in range(0, nh, 256):
                rs, cs = slice(r, r + 8), slice(c0, c0 + 256)
                b11, b21, b22, b12 = [src[q, rs, cs] for q in (0, 1, 2, s12)]
                outs = []
                for idx in (0, 1):
                    a11, a21, a22, a12 = [
                        pltpu.unpack_elementwise(u, index=idx, packed_dtype=BF16, unpacked_dtype=F32)
                        for u in (b11, b21, b22, b12)]
                    t1 = a12 - a11
                    t2 = a22 - t1
                    outs.append((t1, t2, a22 - a12, t2 - a21))
                for q, lo, hi in zip(dsl, *outs):
                    dst[q, rs, cs] = pltpu.pack_elementwise([lo, hi], packed_dtype=BF16)

    def store_q(r0, ys):
        for y, r in zip(ys, (r0, r0 + ys[0].shape[0])):
            qraw[pl.ds(_mo(r // 2, 8), y.shape[0] // 2), :] = _pk(y)

    def store_kv(buf, r0, ys):
        for y, r in zip(ys, (r0, r0 + ys[0].shape[0])):
            yb = _pk(y)
            zs = _butterfly([yb[:, j * 128:(j + 1) * 128] for j in range(NSL)])
            for j in range(NSL):
                buf[j, pl.ds(r + HALO, y.shape[0]), :] = _unpk(zs[j])

    def attn_block(rr, masked):
        lane = lax.broadcasted_iota(I32, (RB, 128), 1)
        i16 = lane ^ 16
        i8 = lane ^ 8
        qh = _mo(rr // 2, RB // 2)
        qr = qraw[pl.ds(qh, RB // 2), :]
        q = [_unpk(u) for u in _butterfly([qr[:, j * 128:(j + 1) * 128] for j in range(NSL)])]
        lg = []
        for w in range(W):
            acc = None
            for j in range(NSL):
                t = q[j] * kbuf[j, pl.ds(rr + HALO - DIL * w, RB), :]
                acc = t if acc is None else acc + t
            acc = acc + jnp.take_along_axis(acc, i16, axis=1)
            acc = acc + jnp.take_along_axis(acc, i8, axis=1)
            if w > 0 and masked:
                pos = rr + lax.broadcasted_iota(I32, (RB, 128), 0)
                acc = jnp.where(pos >= DIL * w, acc, -1e9 * LOG2E)
            lg.append(acc)
        mx = functools.reduce(jnp.maximum, lg)
        es = [jnp.exp2(l - mx) for l in lg]
        rz = 1.0 / functools.reduce(lambda a, b: a + b, es)
        ps = [e * rz for e in es]
        os_ = []
        for j in range(NSL):
            acc = None
            for w in range(W):
                t = ps[w] * vbuf[j, pl.ds(rr + HALO - DIL * w, RB), :]
                acc = t if acc is None else acc + t
            os_.append(acc)
        ob = _butterfly([_u32(u.astype(BF16)) for u in os_])
        obuf[pl.ds(qh, RB // 2), :] = jnp.concatenate(ob, axis=1)

    cp_x0.wait()
    h0 = T0 // 2
    xn = [_ln_norm(x_v[b * 16:(b + 1) * 16, :].astype(F32)) for b in range(T0 // 16)]
    cp_wm[1].wait()
    do_mod(1)
    for cp in kcs[0]:
        cp.wait()
    for b in range(h0 // 16):
        top = xn[b] * mod(1)
        bot = xn[h0 // 16 + b] * mod(1)
        rs = slice(b * 8, (b + 1) * 8)
        for q, u in enumerate((top[:, 0:NH], top[:, NH:], bot[:, 0:NH], bot[:, NH:])):
            hk[q, rs, :] = _u32(u.astype(BF16))
        ops = _a_ops(top[:, 0:NH], top[:, NH:], bot[:, 0:NH], bot[:, NH:])
        for q, p in enumerate((2, 4, 5, 6)):
            hs[q, rs, :] = _u32(ops[p].astype(BF16))

    def hfirst(p):
        return hk[(0, 1, None, 3)[p]] if p in (0, 1, 3) else hs[(2, 4, 5, 6).index(p)]

    def kdot(cl, cr, cs):
        dd = lambda a, q: _dot(_bf(hk[a]), _bf(wr_v[1, q, :, cs]))
        return dd(0, cl) + dd(1, cr), dd(2, cl) + dd(3, cr)

    ytop, ybot = [], []
    for n, (lo, hi) in enumerate(zip(KCH[:-1], KCH[1:])):
        if n > 0:
            for cp in kcs[n]:
                cp.wait()
        a, b = kdot(0, 1, slice(lo, hi))
        ytop.append(a)
        ybot.append(b)
    for cp in kcs[-1]:
        cp.wait()
    a, b = kdot(3, 2, slice(None))
    yk = (jnp.concatenate(ytop + [a], axis=1), jnp.concatenate(ybot + [b], axis=1))
    cp_wm[0].wait()
    do_mod(0)
    for cp in cp_wv:
        cp.wait()
    precompute(wr_v.at[2], wt_v.at[2], QR, NH, 3, (1, 2, 3, 0))
    bias(2)
    yv = proj(hfirst, 2)
    store_kv(kbuf, 0, yk)
    cp_xn.wait()
    for cp in cp_wq:
        cp.wait()
    precompute(wr_v.at[0], wt_v.at[0], QR, NH, 3, (1, 2, 3, 0))
    precompute(wr_v.at[1], wt_v.at[1], QR, NH, 3, (1, 2, 3, 0))
    bias(0)
    for q, u in enumerate(ln1_ops(T0, T1)):
        hbuf[q] = u
    yq = proj(hfirst, 0)
    store_kv(vbuf, 0, yv)
    store_q(0, yq)
    cp_xr.wait()

    def body_a(i, carry):
        r0 = pl.multiple_of(T0 + i * T1, 16)
        rn = pl.multiple_of(jnp.minimum(T0 + (i + 1) * T1, S - T1), 16)
        hop = lambda p: hbuf[p]

        def att(b):
            attn_block(pl.multiple_of((i * NB1 + b) * RB, RB), True)

        yk = proj(hop, 1)
        att(0)
        store_kv(kbuf, r0, yk)
        yv = proj(hop, 2)
        att(1)
        store_kv(vbuf, r0, yv)
        hn = ln1_ops(rn, T1)
        yq = proj(hop, 0)
        for b in range(2, NB1):
            att(b)
        store_q(r0, yq)
        for q, u in enumerate(hn):
            hbuf[q] = u
        return carry

    lax.fori_loop(0, N1, body_a, 0)

    for j in range(2, 6):
        cp_wm[j].wait()
    cp_wo.wait()
    for cp in cp_ffn:
        cp.wait()
    for j in range(2, 6):
        do_mod(j)
    precompute(w1_v, w1_v, D // 4, F // 2, 4, (4, 5, 6, 3))
    precompute(w3_v, w3_v, D // 4, F // 2, 4, (4, 5, 6, 3))
    precompute(w2_v, w2_v, F // 4, D // 2, 4, (4, 5, 6, 3))

    def out_copy(r0):
        return mac(o_v.at[pl.ds(r0, TM), :], o_h.at[pl.ds(r0, TM), :], osem)

    def body_b(i, carry):
        r0 = pl.multiple_of(i * TM, TM)
        rh = pl.multiple_of(i * (TM // 2), TM // 2)
        x1s, h2s = [], []
        for s in range(2):
            ob = _bf(obuf[pl.ds(rh + s * (HM // 2), HM // 2), :])
            x1 = x_v[pl.ds(r0 + s * HM, HM), :].astype(F32) + mod(2) * _dot(ob, _bf(wo_v[...]))
            x1s.append(x1)
            h2s.append(_ln_norm(x1) * mod(4) + mod(3))
        sops = [u.astype(BF16) for u in
                _a_ops(h2s[0][:, 0:NH], h2s[0][:, NH:], h2s[1][:, 0:NH], h2s[1][:, NH:])]
        accs = [None] * 7
        blk = 0
        for f in range(NCH):
            fs = slice(f * SN, (f + 1) * SN)
            g = _c_quads([_dot(sops[p], _bf(w1_v[p, :, fs])) for p in range(7)])
            u = _c_quads([_dot(sops[p], _bf(w3_v[p, :, fs])) for p in range(7)])
            act = []
            for gg, uu in zip(g, u):
                hg = 0.5 * gg
                act.append((hg + hg * jnp.tanh(hg)) * uu)
            aops = [v.astype(BF16) for v in _a_ops(*act)]
            for _ in range(SCH[f]):
                attn_block(pl.multiple_of(
                    jnp.minimum((i + 1) * NBLK + blk, S // RB - 1) * RB, RB), False)
                blk += 1
            for p in range(7):
                t = _dot(aops[p], _bf(w2_v[p, f * SN // 2:(f + 1) * SN // 2, :]))
                accs[p] = t if accs[p] is None else accs[p] + t
        c11, c12, c21, c22 = _c_quads(accs)
        g5 = mod(5)
        o_v[pl.ds(r0, HM), 0:NH] = (x1s[0][:, 0:NH] + g5[:, 0:NH] * c11).astype(BF16)
        o_v[pl.ds(r0, HM), NH:] = (x1s[0][:, NH:] + g5[:, NH:] * c12).astype(BF16)
        o_v[pl.ds(r0 + HM, HM), 0:NH] = (x1s[1][:, 0:NH] + g5[:, 0:NH] * c21).astype(BF16)
        o_v[pl.ds(r0 + HM, HM), NH:] = (x1s[1][:, NH:] + g5[:, NH:] * c22).astype(BF16)
        out_copy(r0).start()
        return carry

    lax.fori_loop(0, NT, body_b, 0)
    for i in range(NT):
        out_copy(i * TM).wait()


@jax.jit
def pallas_adaLN_cond__sliding_local_dilated__glu_gated_swiglu__prompt_kernel(
    A_x: jax.Array,
    A_wqkv: jax.Array,
    A_wo: jax.Array,
    B_x: jax.Array,
    B_w1: jax.Array,
    B_w3: jax.Array,
    B_w2: jax.Array,
    c: jax.Array,
    w_mod: jax.Array,
):
    del B_x
    anyspec = pl.BlockSpec(memory_space=pl.ANY)
    out = pl.pallas_call(
        _kernel,
        in_specs=[anyspec] * 8,
        out_specs=anyspec,
        out_shape=jax.ShapeDtypeStruct((S, D), BF16),
        scratch_shapes=[
            pltpu.VMEM((S, D), BF16),
            pltpu.VMEM((1, D), BF16),
            pltpu.VMEM((3, 4, QR, NH), U32),
            pltpu.VMEM((3, 4, QR, NH), U32),
            pltpu.VMEM((D // 2, D), U32),
            pltpu.VMEM((7, D // 4, F // 2), U32),
            pltpu.VMEM((7, D // 4, F // 2), U32),
            pltpu.VMEM((7, F // 4, D // 2), U32),
            pltpu.VMEM((6, D // 2, D), U32),
            pltpu.VMEM((6, 16, D), F32),
            pltpu.VMEM((2, 8, D), F32),
            pltpu.VMEM((S // 2, D), U32),
            pltpu.VMEM((NSL, S + HALO, 128), F32),
            pltpu.VMEM((NSL, S + HALO, 128), F32),
            pltpu.VMEM((7, T1 // 4, NH), U32),
            pltpu.VMEM((4, T0 // 4, NH), U32),
            pltpu.VMEM((4, T0 // 4, NH), U32),
            pltpu.VMEM((S // 2, D), U32),
            pltpu.VMEM((S, D), BF16),
            pltpu.SemaphoreType.DMA((28,)),
            pltpu.SemaphoreType.DMA(()),
        ],
        compiler_params=pltpu.CompilerParams(vmem_limit_bytes=120 * 1024 * 1024),
    )(A_x.reshape(S, D), c, A_wqkv, A_wo, B_w1, B_w3, B_w2, w_mod)
    return out.reshape(1, S, D)
```

```python
import functools

import jax
import jax.numpy as jnp
from jax import lax
import jax.experimental.pallas as pl
import jax.experimental.pallas.tpu as pltpu

S, D, H, DH, F = 2048, 1024, 32, 32, 3584
W, DIL = 8, 2
HALO = 16
EPS = 1e-5
LOG2E = 1.4426950408889634
QS = DH ** -0.5 * LOG2E
NSL = D // 128
F32, BF16, U32, I32 = jnp.float32, jnp.bfloat16, jnp.uint32, jnp.int32

TM = 256
HM = TM // 2
RB = 16
SN = 256
PC = 256
T0 = 640
N1 = 4
T1 = (S - T0) // N1
KCH = (0, 128, 512)
NT = S // TM
NBLK = TM // RB
NB1 = NBLK // N1
NCH = (F // 2) // SN
SCH = [NBLK // NCH + (1 if f < NBLK % NCH else 0) for f in range(NCH)]
QR, NH = D // 4, D // 2


def _butterfly(xs):
    lane = lax.broadcasted_iota(I32, xs[0].shape, 1)
    for b in (4, 2, 1):
        m = (lane & b) != 0
        ys = list(xs)
        for j in range(8):
            if j & b == 0:
                lo, hi = xs[j], xs[j | b]
                ys[j] = jnp.where(m, pltpu.roll(hi, b, 1), lo)
                ys[j | b] = jnp.where(m, hi, pltpu.roll(lo, 128 - b, 1))
        xs = ys
    return xs


def _a_ops(a11, a12, a21, a22):
    s1 = a21 + a22
    s2 = s1 - a11
    return [a11, a12, a12 - s2, a22, s1, s2, a11 - a21]


def _c_quads(p):
    p1, p2, p3, p4, p5, p6, p7 = p
    u2 = p1 + p6
    u3 = u2 + p7
    return p1 + p2, (u2 + p5) + p3, u3 - p4, u3 + p5


def _ln_norm(xf):
    m = jnp.mean(xf, axis=-1, keepdims=True)
    xc = xf - m
    v = jnp.mean(xc * xc, axis=-1, keepdims=True)
    return xc * lax.rsqrt(v + EPS)


def _bf(u):
    return pltpu.bitcast(u, BF16)


def _u32(b):
    return pltpu.bitcast(b, U32)


def _pk(y):
    r = y.shape[0]
    lo = jnp.concatenate([y[g:g + 8] for g in range(0, r, 16)], axis=0)
    hi = jnp.concatenate([y[g + 8:g + 16] for g in range(0, r, 16)], axis=0)
    return pltpu.pack_elementwise([lo, hi], packed_dtype=BF16)


def _unpk(u):
    lo = pltpu.unpack_elementwise(u, index=0, packed_dtype=BF16, unpacked_dtype=F32)
    hi = pltpu.unpack_elementwise(u, index=1, packed_dtype=BF16, unpacked_dtype=F32)
    parts = []
    for g in range(0, u.shape[0], 8):
        parts += [lo[g:g + 8], hi[g:g + 8]]
    return jnp.concatenate(parts, axis=0)


def _mo(v, m):
    return v if isinstance(v, int) else pl.multiple_of(v, m)


def _dot(a, b):
    return jnp.dot(a, b, preferred_element_type=F32)


def _kernel(x_h, c_h, wqkv_h, wo_h, w1_h, w3_h, w2_h, wm_h, o_h,
            x_v, c_v, wr_v, wt_v, w1_v, w3_v, w2_v, wm_v, mod_v, bias_v,
            qraw, kbuf, vbuf, hbuf, hk, hs, obuf, o_v, sems, osem):
    wqkv_u, wo_u, w1_u, w3_u, w2_u, wm_u = [
        r.bitcast(U32) for r in (wqkv_h, wo_h, w1_h, w3_h, w2_h, wm_h)]
    mac = pltpu.make_async_copy

    cp_c = mac(c_h, c_v, sems.at[0])
    cp_x0 = mac(x_h.at[0:T0, :], x_v.at[0:T0, :], sems.at[1])
    cp_xn = mac(x_h.at[T0:T0 + T1, :], x_v.at[T0:T0 + T1, :], sems.at[2])
    cp_xr = mac(x_h.at[T0 + T1:S, :], x_v.at[T0 + T1:S, :], sems.at[3])
    cp_wm = [mac(wm_u.at[:, j * D:(j + 1) * D], wm_v.at[j], sems.at[4 + j]) for j in range(6)]

    def quad(t, slot, lo=0, hi=NH):
        ro, co = ((0, 0), (QR, 0), (QR, NH), (0, NH))[slot]
        return (wqkv_u.at[ro:ro + QR, t * D + co + lo:t * D + co + hi], wr_v.at[t, slot, :, lo:hi])

    kcs = [[mac(*quad(1, 0, lo, hi), sems.at[10 + n]), mac(*quad(1, 1, lo, hi), sems.at[10 + n])]
           for n, (lo, hi) in enumerate(zip(KCH[:-1], KCH[1:]))]
    kcs.append([mac(*quad(1, 3), sems.at[12]), mac(*quad(1, 2), sems.at[12])])
    cp_wv = [mac(*quad(2, q), sems.at[13]) for q in range(4)]
    cp_wq = [mac(*quad(0, q), sems.at[14]) for q in range(4)]
    cp_wo = [mac(wo_u.at[ro:ro + QR, co:co + NH], wr_v.at[3, q], sems.at[15])
             for q, (ro, co) in enumerate(((0, 0), (QR, 0), (QR, NH), (0, NH)))]

    def wcopies(src, dst, kh, nh, base):
        return [mac(src.at[0:kh, 0:nh], dst.at[0], sems.at[base]),
                mac(src.at[kh:2 * kh, 0:nh], dst.at[1], sems.at[base + 1]),
                mac(src.at[kh:2 * kh, nh:2 * nh], dst.at[2], sems.at[base + 2]),
                mac(src.at[0:kh, nh:2 * nh], dst.at[4], sems.at[base + 3])]

    cp_ffn = (wcopies(w1_u, w1_v, D // 4, F // 2, 16) + wcopies(w3_u, w3_v, D // 4, F // 2, 20)
              + wcopies(w2_u, w2_v, F // 4, D // 2, 24))
    for cp in ([cp_c, cp_x0, cp_wm[1]] + sum(kcs, []) + [cp_wm[0]] + cp_wv + [cp_xn] + cp_wq
               + [cp_xr, cp_wm[2], cp_wm[3], cp_wm[4], cp_wm[5]] + cp_wo + cp_ffn):
        cp.start()

    kbuf[:, 0:HALO, :] = jnp.zeros((NSL, HALO, 128), F32)
    vbuf[:, 0:HALO, :] = jnp.zeros((NSL, HALO, 128), F32)
    cp_c.wait()
    cf = c_v[...].astype(F32)
    sc = jnp.broadcast_to((cf * jax.nn.sigmoid(cf)).astype(BF16), (16, D))

    def do_mod(j):
        r = _dot(sc, _bf(wm_v[j]))
        mod_v[j] = 1.0 + r if j in (1, 4) else r

    def mod(j):
        return mod_v[j, 0:1, :]

    def ln1_ops(r0, rows):
        half = rows // 2
        outs = [[] for _ in range(7)]
        for b in range(half // 16):
            top = _ln_norm(x_v[pl.ds(r0 + b * 16, 16), :].astype(F32)) * mod(1)
            bot = _ln_norm(x_v[pl.ds(r0 + half + b * 16, 16), :].astype(F32)) * mod(1)
            for q, u in enumerate(_a_ops(top[:, 0:NH], top[:, NH:], bot[:, 0:NH], bot[:, NH:])):
                outs[q].append(_u32(u.astype(BF16)))
        return [jnp.concatenate(o, axis=0) for o in outs]

    def bias(t):
        sa = mod_v[0].astype(BF16)
        dd = lambda cs, q: _dot(sa[:, cs], _bf(wr_v[t, q]))
        lo, hi = slice(0, NH), slice(NH, D)
        b = jnp.concatenate([dd(lo, 0) + dd(hi, 1), dd(lo, 3) + dd(hi, 2)], axis=1)[0:8, :]
        bias_v[t // 2] = b * QS if t == 0 else b

    def proj(hop, t):
        def wop(p, cs):
            return _bf(wr_v[t, p, :, cs] if p < 3 else wt_v[t, p - 3, :, cs])
        parts = [_c_quads([_dot(_bf(hop(p)), wop(p, slice(c0, c0 + PC))) for p in range(7)])
                 for c0 in range(0, NH, PC)]
        c11, c12, c21, c22 = [jnp.concatenate([pp[q] for pp in parts], axis=1) for q in range(4)]
        top = jnp.concatenate([c11, c12], axis=1)
        bot = jnp.concatenate([c21, c22], axis=1)
        if t == 1:
            return top, bot
        b = bias_v[t // 2, 0:1, :]
        return (top * QS + b, bot * QS + b) if t == 0 else (top + b, bot + b)

    def precompute(src, dst, kh, nh, s12, dsl):
        for r in range(0, kh, 8):
            for c0 in range(0, nh, 256):
                rs, cs = slice(r, r + 8), slice(c0, c0 + 256)
                b11, b21, b22, b12 = [src[q, rs, cs] for q in (0, 1, 2, s12)]
                outs = []
                for idx in (0, 1):
                    a11, a21, a22, a12 = [
                        pltpu.unpack_elementwise(u, index=idx, packed_dtype=BF16, unpacked_dtype=F32)
                        for u in (b11, b21, b22, b12)]
                    t1 = a12 - a11
                    t2 = a22 - t1
                    outs.append((t1, t2, a22 - a12, t2 - a21))
                for q, lo, hi in zip(dsl, *outs):
                    dst[q, rs, cs] = pltpu.pack_elementwise([lo, hi], packed_dtype=BF16)

    def store_q(r0, ys):
        for y, r in zip(ys, (r0, r0 + ys[0].shape[0])):
            qraw[pl.ds(_mo(r // 2, 8), y.shape[0] // 2), :] = _pk(y)

    def store_kv(buf, r0, ys):
        for y, r in zip(ys, (r0, r0 + ys[0].shape[0])):
            yb = _pk(y)
            zs = _butterfly([yb[:, j * 128:(j + 1) * 128] for j in range(NSL)])
            for j in range(NSL):
                buf[j, pl.ds(r + HALO, y.shape[0]), :] = _unpk(zs[j])

    def attn_block(rr, masked):
        lane = lax.broadcasted_iota(I32, (RB, 128), 1)
        i16 = lane ^ 16
        i8 = lane ^ 8
        qh = _mo(rr // 2, RB // 2)
        qr = qraw[pl.ds(qh, RB // 2), :]
        q = [_unpk(u) for u in _butterfly([qr[:, j * 128:(j + 1) * 128] for j in range(NSL)])]
        lg = []
        for w in range(W):
            acc = None
            for j in range(NSL):
                t = q[j] * kbuf[j, pl.ds(rr + HALO - DIL * w, RB), :]
                acc = t if acc is None else acc + t
            acc = acc + jnp.take_along_axis(acc, i16, axis=1)
            acc = acc + jnp.take_along_axis(acc, i8, axis=1)
            if w > 0 and masked:
                pos = rr + lax.broadcasted_iota(I32, (RB, 128), 0)
                acc = jnp.where(pos >= DIL * w, acc, -1e9 * LOG2E)
            lg.append(acc)
        mx = functools.reduce(jnp.maximum, lg)
        es = [jnp.exp2(l - mx) for l in lg]
        rz = 1.0 / functools.reduce(lambda a, b: a + b, es)
        ps = [e * rz for e in es]
        os_ = []
        for j in range(NSL):
            acc = None
            for w in range(W):
                t = ps[w] * vbuf[j, pl.ds(rr + HALO - DIL * w, RB), :]
                acc = t if acc is None else acc + t
            os_.append(acc)
        ob = _butterfly([_u32(u.astype(BF16)) for u in os_])
        obuf[pl.ds(qh, RB // 2), :] = jnp.concatenate(ob, axis=1)

    cp_x0.wait()
    h0 = T0 // 2
    xn = [_ln_norm(x_v[b * 16:(b + 1) * 16, :].astype(F32)) for b in range(T0 // 16)]
    cp_wm[1].wait()
    do_mod(1)
    for cp in kcs[0]:
        cp.wait()
    for b in range(h0 // 16):
        top = xn[b] * mod(1)
        bot = xn[h0 // 16 + b] * mod(1)
        rs = slice(b * 8, (b + 1) * 8)
        for q, u in enumerate((top[:, 0:NH], top[:, NH:], bot[:, 0:NH], bot[:, NH:])):
            hk[q, rs, :] = _u32(u.astype(BF16))
        ops = _a_ops(top[:, 0:NH], top[:, NH:], bot[:, 0:NH], bot[:, NH:])
        for q, p in enumerate((2, 4, 5, 6)):
            hs[q, rs, :] = _u32(ops[p].astype(BF16))

    def hfirst(p):
        return hk[(0, 1, None, 3)[p]] if p in (0, 1, 3) else hs[(2, 4, 5, 6).index(p)]

    def kdot(cl, cr, cs):
        dd = lambda a, q: _dot(_bf(hk[a]), _bf(wr_v[1, q, :, cs]))
        return dd(0, cl) + dd(1, cr), dd(2, cl) + dd(3, cr)

    ytop, ybot = [], []
    for n, (lo, hi) in enumerate(zip(KCH[:-1], KCH[1:])):
        if n > 0:
            for cp in kcs[n]:
                cp.wait()
        a, b = kdot(0, 1, slice(lo, hi))
        ytop.append(a)
        ybot.append(b)
    for cp in kcs[-1]:
        cp.wait()
    a, b = kdot(3, 2, slice(None))
    yk = (jnp.concatenate(ytop + [a], axis=1), jnp.concatenate(ybot + [b], axis=1))
    cp_wm[0].wait()
    do_mod(0)
    for cp in cp_wv:
        cp.wait()
    precompute(wr_v.at[2], wt_v.at[2], QR, NH, 3, (1, 2, 3, 0))
    bias(2)
    yv = proj(hfirst, 2)
    store_kv(kbuf, 0, yk)
    cp_xn.wait()
    for cp in cp_wq:
        cp.wait()
    precompute(wr_v.at[0], wt_v.at[0], QR, NH, 3, (1, 2, 3, 0))
    precompute(wr_v.at[1], wt_v.at[1], QR, NH, 3, (1, 2, 3, 0))
    bias(0)
    for q, u in enumerate(ln1_ops(T0, T1)):
        hbuf[q] = u
    yq = proj(hfirst, 0)
    store_kv(vbuf, 0, yv)
    store_q(0, yq)
    cp_xr.wait()

    def body_a(i, carry):
        r0 = pl.multiple_of(T0 + i * T1, 16)
        rn = pl.multiple_of(jnp.minimum(T0 + (i + 1) * T1, S - T1), 16)
        hop = lambda p: hbuf[p]

        def att(b):
            attn_block(pl.multiple_of((i * NB1 + b) * RB, RB), True)

        yk = proj(hop, 1)
        att(0)
        store_kv(kbuf, r0, yk)
        yv = proj(hop, 2)
        att(1)
        store_kv(vbuf, r0, yv)
        hn = ln1_ops(rn, T1)
        yq = proj(hop, 0)
        for b in range(2, NB1):
            att(b)
        store_q(r0, yq)
        for q, u in enumerate(hn):
            hbuf[q] = u
        return carry

    lax.fori_loop(0, N1, body_a, 0)

    for j in range(2, 6):
        cp_wm[j].wait()
    for cp in cp_wo:
        cp.wait()
    for cp in cp_ffn:
        cp.wait()
    for j in range(2, 6):
        do_mod(j)
    precompute(wr_v.at[3], wt_v.at[3], QR, NH, 3, (1, 2, 3, 0))
    precompute(w1_v, w1_v, D // 4, F // 2, 4, (4, 5, 6, 3))
    precompute(w3_v, w3_v, D // 4, F // 2, 4, (4, 5, 6, 3))
    precompute(w2_v, w2_v, F // 4, D // 2, 4, (4, 5, 6, 3))

    def out_copy(r0):
        return mac(o_v.at[pl.ds(r0, TM), :], o_h.at[pl.ds(r0, TM), :], osem)

    def body_b(i, carry):
        r0 = pl.multiple_of(i * TM, TM)
        rh = pl.multiple_of(i * (TM // 2), TM // 2)
        ot = _bf(obuf[pl.ds(rh, HM // 2), :]).astype(F32)
        ob = _bf(obuf[pl.ds(rh + HM // 2, HM // 2), :]).astype(F32)
        oo = [u.astype(BF16) for u in _a_ops(ot[:, 0:NH], ot[:, NH:], ob[:, 0:NH], ob[:, NH:])]
        cq = _c_quads([_dot(oo[p], _bf(wr_v[3, p] if p < 3 else wt_v[3, p - 3])) for p in range(7)])
        x1s, h2s = [], []
        for s in range(2):
            a = jnp.concatenate([cq[2 * s], cq[2 * s + 1]], axis=1)
            x1 = x_v[pl.ds(r0 + s * HM, HM), :].astype(F32) + mod(2) * a
            x1s.append(x1)
            h2s.append(_ln_norm(x1) * mod(4) + mod(3))
        sops = [u.astype(BF16) for u in
                _a_ops(h2s[0][:, 0:NH], h2s[0][:, NH:], h2s[1][:, 0:NH], h2s[1][:, NH:])]
        accs = [None] * 7
        blk = 0
        for f in range(NCH):
            fs = slice(f * SN, (f + 1) * SN)
            g = _c_quads([_dot(sops[p], _bf(w1_v[p, :, fs])) for p in range(7)])
            u = _c_quads([_dot(sops[p], _bf(w3_v[p, :, fs])) for p in range(7)])
            act = []
            for gg, uu in zip(g, u):
                hg = 0.5 * gg
                act.append((hg + hg * jnp.tanh(hg)) * uu)
            aops = [v.astype(BF16) for v in _a_ops(*act)]
            for _ in range(SCH[f]):
                attn_block(pl.multiple_of(
                    jnp.minimum((i + 1) * NBLK + blk, S // RB - 1) * RB, RB), False)
                blk += 1
            for p in range(7):
                t = _dot(aops[p], _bf(w2_v[p, f * SN // 2:(f + 1) * SN // 2, :]))
                accs[p] = t if accs[p] is None else accs[p] + t
        c11, c12, c21, c22 = _c_quads(accs)
        g5 = mod(5)
        o_v[pl.ds(r0, HM), 0:NH] = (x1s[0][:, 0:NH] + g5[:, 0:NH] * c11).astype(BF16)
        o_v[pl.ds(r0, HM), NH:] = (x1s[0][:, NH:] + g5[:, NH:] * c12).astype(BF16)
        o_v[pl.ds(r0 + HM, HM), 0:NH] = (x1s[1][:, 0:NH] + g5[:, 0:NH] * c21).astype(BF16)
        o_v[pl.ds(r0 + HM, HM), NH:] = (x1s[1][:, NH:] + g5[:, NH:] * c22).astype(BF16)
        out_copy(r0).start()
        return carry

    lax.fori_loop(0, NT, body_b, 0)
    for i in range(NT):
        out_copy(i * TM).wait()


@jax.jit
def pallas_adaLN_cond__sliding_local_dilated__glu_gated_swiglu__prompt_kernel(
    A_x: jax.Array,
    A_wqkv: jax.Array,
    A_wo: jax.Array,
    B_x: jax.Array,
    B_w1: jax.Array,
    B_w3: jax.Array,
    B_w2: jax.Array,
    c: jax.Array,
    w_mod: jax.Array,
):
    del B_x
    anyspec = pl.BlockSpec(memory_space=pl.ANY)
    out = pl.pallas_call(
        _kernel,
        in_specs=[anyspec] * 8,
        out_specs=anyspec,
        out_shape=jax.ShapeDtypeStruct((S, D), BF16),
        scratch_shapes=[
            pltpu.VMEM((S, D), BF16),
            pltpu.VMEM((1, D), BF16),
            pltpu.VMEM((4, 4, QR, NH), U32),
            pltpu.VMEM((4, 4, QR, NH), U32),
            pltpu.VMEM((7, D // 4, F // 2), U32),
            pltpu.VMEM((7, D // 4, F // 2), U32),
            pltpu.VMEM((7, F // 4, D // 2), U32),
            pltpu.VMEM((6, D // 2, D), U32),
            pltpu.VMEM((6, 16, D), F32),
            pltpu.VMEM((2, 8, D), F32),
            pltpu.VMEM((S // 2, D), U32),
            pltpu.VMEM((NSL, S + HALO, 128), F32),
            pltpu.VMEM((NSL, S + HALO, 128), F32),
            pltpu.VMEM((7, T1 // 4, NH), U32),
            pltpu.VMEM((4, T0 // 4, NH), U32),
            pltpu.VMEM((4, T0 // 4, NH), U32),
            pltpu.VMEM((S // 2, D), U32),
            pltpu.VMEM((S, D), BF16),
            pltpu.SemaphoreType.DMA((28,)),
            pltpu.SemaphoreType.DMA(()),
        ],
        compiler_params=pltpu.CompilerParams(
            vmem_limit_bytes=120 * 1024 * 1024,
            flags={"XLA_TPU_EVENLY_DISTRIBUTE_CRITICAL_NODES": True}),
    )(A_x.reshape(S, D), c, A_wqkv, A_wo, B_w1, B_w3, B_w2, w_mod)
    return out.reshape(1, S, D)
```

```python
import functools

import jax
import jax.numpy as jnp
from jax import lax
import jax.experimental.pallas as pl
import jax.experimental.pallas.tpu as pltpu

S, D, H, DH, F = 2048, 1024, 32, 32, 3584
W, DIL = 8, 2
HALO = 16
EPS = 1e-5
LOG2E = 1.4426950408889634
QS = DH ** -0.5 * LOG2E
NSL = D // 128
F32, BF16, U32, I32 = jnp.float32, jnp.bfloat16, jnp.uint32, jnp.int32

TM = 256
HM = TM // 2
RB = 16
SN = 256
PC = 256
T0 = 640
N1 = 4
T1 = (S - T0) // N1
KCH = (0, 128, 512)
NT = S // TM
NBLK = TM // RB
NB1 = NBLK // N1
NCH = (F // 2) // SN
SCH = [NBLK // NCH + (1 if f < NBLK % NCH else 0) for f in range(NCH)]
QR, NH = D // 4, D // 2


def _butterfly(xs):
    lane = lax.broadcasted_iota(I32, xs[0].shape, 1)
    for b in (4, 2, 1):
        m = (lane & b) != 0
        ys = list(xs)
        for j in range(8):
            if j & b == 0:
                lo, hi = xs[j], xs[j | b]
                ys[j] = jnp.where(m, pltpu.roll(hi, b, 1), lo)
                ys[j | b] = jnp.where(m, hi, pltpu.roll(lo, 128 - b, 1))
        xs = ys
    return xs


def _a_ops(a11, a12, a21, a22):
    s1 = a21 + a22
    s2 = s1 - a11
    return [a11, a12, a12 - s2, a22, s1, s2, a11 - a21]


def _c_quads(p):
    p1, p2, p3, p4, p5, p6, p7 = p
    u2 = p1 + p6
    u3 = u2 + p7
    return p1 + p2, (u2 + p5) + p3, u3 - p4, u3 + p5


def _ln_norm(xf):
    m = jnp.mean(xf, axis=-1, keepdims=True)
    xc = xf - m
    v = jnp.mean(xc * xc, axis=-1, keepdims=True)
    return xc * lax.rsqrt(v + EPS)


def _bf(u):
    return pltpu.bitcast(u, BF16)


def _u32(b):
    return pltpu.bitcast(b, U32)


def _pk(y):
    r = y.shape[0]
    lo = jnp.concatenate([y[g:g + 8] for g in range(0, r, 16)], axis=0)
    hi = jnp.concatenate([y[g + 8:g + 16] for g in range(0, r, 16)], axis=0)
    return pltpu.pack_elementwise([lo, hi], packed_dtype=BF16)


def _unpk(u):
    lo = pltpu.unpack_elementwise(u, index=0, packed_dtype=BF16, unpacked_dtype=F32)
    hi = pltpu.unpack_elementwise(u, index=1, packed_dtype=BF16, unpacked_dtype=F32)
    parts = []
    for g in range(0, u.shape[0], 8):
        parts += [lo[g:g + 8], hi[g:g + 8]]
    return jnp.concatenate(parts, axis=0)


def _mo(v, m):
    return v if isinstance(v, int) else pl.multiple_of(v, m)


def _dot(a, b):
    return jnp.dot(a, b, preferred_element_type=F32)


def _kernel(x_h, c_h, wqkv_h, wo_h, w1_h, w3_h, w2_h, wm_h, o_h,
            x_v, c_v, wr_v, wt_v, w1_v, w3_v, w2_v, wm_v, mod_v, bias_v,
            qraw, kbuf, vbuf, hbuf, hk, hs, obuf, o_v, sems, osem):
    wqkv_u, wo_u, w1_u, w3_u, w2_u, wm_u = [
        r.bitcast(U32) for r in (wqkv_h, wo_h, w1_h, w3_h, w2_h, wm_h)]
    mac = pltpu.make_async_copy

    cp_c = mac(c_h, c_v, sems.at[0])
    cp_x0 = mac(x_h.at[0:T0, :], x_v.at[0:T0, :], sems.at[1])
    cp_xn = mac(x_h.at[T0:T0 + T1, :], x_v.at[T0:T0 + T1, :], sems.at[2])
    cp_xr = mac(x_h.at[T0 + T1:S, :], x_v.at[T0 + T1:S, :], sems.at[3])
    cp_wm = [mac(wm_u.at[:, j * D:(j + 1) * D], wm_v.at[j], sems.at[4 + j]) for j in range(6)]

    def quad(t, slot, lo=0, hi=NH):
        ro, co = ((0, 0), (QR, 0), (QR, NH), (0, NH))[slot]
        return (wqkv_u.at[ro:ro + QR, t * D + co + lo:t * D + co + hi], wr_v.at[t, slot, :, lo:hi])

    kcs = [[mac(*quad(1, 0, lo, hi), sems.at[10 + n]), mac(*quad(1, 1, lo, hi), sems.at[10 + n])]
           for n, (lo, hi) in enumerate(zip(KCH[:-1], KCH[1:]))]
    kcs.append([mac(*quad(1, 3), sems.at[12]), mac(*quad(1, 2), sems.at[12])])
    cp_wv = [mac(*quad(2, q), sems.at[13]) for q in range(4)]
    cp_wq = [mac(*quad(0, q), sems.at[14]) for q in range(4)]
    cp_wo = [mac(wo_u.at[ro:ro + QR, co:co + NH], wr_v.at[3, q], sems.at[15])
             for q, (ro, co) in enumerate(((0, 0), (QR, 0), (QR, NH), (0, NH)))]

    def wcopies(src, dst, kh, nh, base):
        return [mac(src.at[0:kh, 0:nh], dst.at[0], sems.at[base]),
                mac(src.at[kh:2 * kh, 0:nh], dst.at[1], sems.at[base + 1]),
                mac(src.at[kh:2 * kh, nh:2 * nh], dst.at[2], sems.at[base + 2]),
                mac(src.at[0:kh, nh:2 * nh], dst.at[4], sems.at[base + 3])]

    cp_ffn = (wcopies(w1_u, w1_v, D // 4, F // 2, 16) + wcopies(w3_u, w3_v, D // 4, F // 2, 20)
              + wcopies(w2_u, w2_v, F // 4, D // 2, 24))
    for cp in ([cp_c, cp_x0, cp_wm[1]] + sum(kcs, []) + [cp_wm[0]] + cp_wv + [cp_xn] + cp_wq
               + [cp_xr, cp_wm[2], cp_wm[3], cp_wm[4], cp_wm[5]] + cp_wo + cp_ffn):
        cp.start()

    kbuf[:, 0:HALO, :] = jnp.zeros((NSL, HALO, 128), F32)
    cp_c.wait()
    cf = c_v[...].astype(F32)
    sc = jnp.broadcast_to((cf * jax.nn.sigmoid(cf)).astype(BF16), (16, D))

    def do_mod(j):
        r = _dot(sc, _bf(wm_v[j]))
        mod_v[j] = 1.0 + r if j in (1, 4) else r

    def mod(j):
        return mod_v[j, 0:1, :]

    def ln1_ops(r0, rows):
        half = rows // 2
        outs = [[] for _ in range(7)]
        for b in range(half // 16):
            top = _ln_norm(x_v[pl.ds(r0 + b * 16, 16), :].astype(F32)) * mod(1)
            bot = _ln_norm(x_v[pl.ds(r0 + half + b * 16, 16), :].astype(F32)) * mod(1)
            for q, u in enumerate(_a_ops(top[:, 0:NH], top[:, NH:], bot[:, 0:NH], bot[:, NH:])):
                outs[q].append(_u32(u.astype(BF16)))
        return [jnp.concatenate(o, axis=0) for o in outs]

    def bias(t):
        sa = mod_v[0].astype(BF16)
        dd = lambda cs, q: _dot(sa[:, cs], _bf(wr_v[t, q]))
        lo, hi = slice(0, NH), slice(NH, D)
        b = jnp.concatenate([dd(lo, 0) + dd(hi, 1), dd(lo, 3) + dd(hi, 2)], axis=1)[0:8, :]
        bias_v[t] = b * QS if t == 0 else b

    def proj(hop, t):
        def wop(p, cs):
            return _bf(wr_v[t, p, :, cs] if p < 3 else wt_v[t, p - 3, :, cs])
        parts = [_c_quads([_dot(_bf(hop(p)), wop(p, slice(c0, c0 + PC))) for p in range(7)])
                 for c0 in range(0, NH, PC)]
        c11, c12, c21, c22 = [jnp.concatenate([pp[q] for pp in parts], axis=1) for q in range(4)]
        top = jnp.concatenate([c11, c12], axis=1)
        bot = jnp.concatenate([c21, c22], axis=1)
        b = bias_v[t, 0:1, :]
        return (top * QS + b, bot * QS + b) if t == 0 else (top + b, bot + b)

    def precompute(src, dst, kh, nh, s12, dsl):
        for r in range(0, kh, 8):
            for c0 in range(0, nh, 256):
                rs, cs = slice(r, r + 8), slice(c0, c0 + 256)
                b11, b21, b22, b12 = [src[q, rs, cs] for q in (0, 1, 2, s12)]
                outs = []
                for idx in (0, 1):
                    a11, a21, a22, a12 = [
                        pltpu.unpack_elementwise(u, index=idx, packed_dtype=BF16, unpacked_dtype=F32)
                        for u in (b11, b21, b22, b12)]
                    t1 = a12 - a11
                    t2 = a22 - t1
                    outs.append((t1, t2, a22 - a12, t2 - a21))
                for q, lo, hi in zip(dsl, *outs):
                    dst[q, rs, cs] = pltpu.pack_elementwise([lo, hi], packed_dtype=BF16)

    def store_q(r0, ys):
        for y, r in zip(ys, (r0, r0 + ys[0].shape[0])):
            qraw[pl.ds(_mo(r // 2, 8), y.shape[0] // 2), :] = _pk(y)

    def store_kv(buf, r0, ys):
        for y, r in zip(ys, (r0, r0 + ys[0].shape[0])):
            yb = _pk(y)
            zs = _butterfly([yb[:, j * 128:(j + 1) * 128] for j in range(NSL)])
            for j in range(NSL):
                buf[j, pl.ds(r + HALO, y.shape[0]), :] = _unpk(zs[j])

    def attn_block(rr, masked):
        lane = lax.broadcasted_iota(I32, (RB, 128), 1)
        i16 = lane ^ 16
        i8 = lane ^ 8
        qh = _mo(rr // 2, RB // 2)
        qr = qraw[pl.ds(qh, RB // 2), :]
        q = [_unpk(u) for u in _butterfly([qr[:, j * 128:(j + 1) * 128] for j in range(NSL)])]
        lg = []
        for w in range(W):
            acc = None
            for j in range(NSL):
                t = q[j] * kbuf[j, pl.ds(rr + HALO - DIL * w, RB), :]
                acc = t if acc is None else acc + t
            acc = acc + jnp.take_along_axis(acc, i16, axis=1)
            acc = acc + jnp.take_along_axis(acc, i8, axis=1)
            if w > 0 and masked:
                pos = rr + lax.broadcasted_iota(I32, (RB, 128), 0)
                acc = jnp.where(pos >= DIL * w, acc, -1e9 * LOG2E)
            lg.append(acc)
        mx = functools.reduce(jnp.maximum, lg)
        es = [jnp.exp2(l - mx) for l in lg]
        rz = 1.0 / functools.reduce(lambda a, b: a + b, es)
        ps = [e * rz for e in es]
        os_ = []
        for j in range(NSL):
            acc = None
            for w in range(W):
                t = ps[w] * vbuf[j, pl.ds(rr + HALO - DIL * w, RB), :]
                acc = t if acc is None else acc + t
            os_.append(acc)
        ob = _butterfly([_u32(u.astype(BF16)) for u in os_])
        obuf[pl.ds(qh, RB // 2), :] = jnp.concatenate(ob, axis=1)

    cp_x0.wait()
    h0 = T0 // 2
    xn = [_ln_norm(x_v[b * 16:(b + 1) * 16, :].astype(F32)) for b in range(T0 // 16)]
    cp_wm[1].wait()
    do_mod(1)
    for cp in kcs[0]:
        cp.wait()
    for b in range(h0 // 16):
        top = xn[b] * mod(1)
        bot = xn[h0 // 16 + b] * mod(1)
        rs = slice(b * 8, (b + 1) * 8)
        for q, u in enumerate((top[:, 0:NH], top[:, NH:], bot[:, 0:NH], bot[:, NH:])):
            hk[q, rs, :] = _u32(u.astype(BF16))
        ops = _a_ops(top[:, 0:NH], top[:, NH:], bot[:, 0:NH], bot[:, NH:])
        for q, p in enumerate((2, 4, 5, 6)):
            hs[q, rs, :] = _u32(ops[p].astype(BF16))

    def hfirst(p):
        return hk[(0, 1, None, 3)[p]] if p in (0, 1, 3) else hs[(2, 4, 5, 6).index(p)]

    def kdot(cl, cr, cs):
        dd = lambda a, q: _dot(_bf(hk[a]), _bf(wr_v[1, q, :, cs]))
        return dd(0, cl) + dd(1, cr), dd(2, cl) + dd(3, cr)

    ytop, ybot = [], []
    for n, (lo, hi) in enumerate(zip(KCH[:-1], KCH[1:])):
        if n > 0:
            for cp in kcs[n]:
                cp.wait()
        a, b = kdot(0, 1, slice(lo, hi))
        ytop.append(a)
        ybot.append(b)
    for cp in kcs[-1]:
        cp.wait()
    a, b = kdot(3, 2, slice(None))
    yk = (jnp.concatenate(ytop + [a], axis=1), jnp.concatenate(ybot + [b], axis=1))
    cp_wm[0].wait()
    do_mod(0)
    for cp in cp_wv:
        cp.wait()
    precompute(wr_v.at[2], wt_v.at[2], QR, NH, 3, (1, 2, 3, 0))
    bias(1)
    bias(2)
    yv = proj(hfirst, 2)
    bk = bias_v[1, 0:1, :]
    store_kv(kbuf, 0, (yk[0] + bk, yk[1] + bk))
    cp_xn.wait()
    for cp in cp_wq:
        cp.wait()
    precompute(wr_v.at[0], wt_v.at[0], QR, NH, 3, (1, 2, 3, 0))
    precompute(wr_v.at[1], wt_v.at[1], QR, NH, 3, (1, 2, 3, 0))
    bias(0)
    for q, u in enumerate(ln1_ops(T0, T1)):
        hbuf[q] = u
    yq = proj(hfirst, 0)
    store_kv(vbuf, 0, yv)
    for j in range(NSL):
        vbuf[j, 0:HALO, :] = jnp.broadcast_to(vbuf[j, HALO:HALO + 1, :], (HALO, 128))
    store_q(0, yq)
    cp_xr.wait()

    def body_a(i, carry):
        r0 = pl.multiple_of(T0 + i * T1, 16)
        rn = pl.multiple_of(jnp.minimum(T0 + (i + 1) * T1, S - T1), 16)
        hop = lambda p: hbuf[p]

        def att(b):
            attn_block(pl.multiple_of((i * NB1 + b) * RB, RB), True)

        yk = proj(hop, 1)
        att(0)
        store_kv(kbuf, r0, yk)
        yv = proj(hop, 2)
        att(1)
        store_kv(vbuf, r0, yv)
        hn = ln1_ops(rn, T1)
        yq = proj(hop, 0)
        for b in range(2, NB1):
            att(b)
        store_q(r0, yq)
        for q, u in enumerate(hn):
            hbuf[q] = u
        return carry

    lax.fori_loop(0, N1, body_a, 0)

    for j in range(2, 6):
        cp_wm[j].wait()
    for cp in cp_wo:
        cp.wait()
    for cp in cp_ffn:
        cp.wait()
    for j in range(2, 6):
        do_mod(j)
    precompute(wr_v.at[3], wt_v.at[3], QR, NH, 3, (1, 2, 3, 0))
    precompute(w1_v, w1_v, D // 4, F // 2, 4, (4, 5, 6, 3))
    precompute(w3_v, w3_v, D // 4, F // 2, 4, (4, 5, 6, 3))
    precompute(w2_v, w2_v, F // 4, D // 2, 4, (4, 5, 6, 3))

    def out_copy(r0):
        return mac(o_v.at[pl.ds(r0, TM), :], o_h.at[pl.ds(r0, TM), :], osem)

    def body_b(i, carry):
        r0 = pl.multiple_of(i * TM, TM)
        rh = pl.multiple_of(i * (TM // 2), TM // 2)
        ot = _bf(obuf[pl.ds(rh, HM // 2), :]).astype(F32)
        ob = _bf(obuf[pl.ds(rh + HM // 2, HM // 2), :]).astype(F32)
        oo = [u.astype(BF16) for u in _a_ops(ot[:, 0:NH], ot[:, NH:], ob[:, 0:NH], ob[:, NH:])]
        cq = _c_quads([_dot(oo[p], _bf(wr_v[3, p] if p < 3 else wt_v[3, p - 3])) for p in range(7)])
        x1s, h2s = [], []
        for s in range(2):
            a = jnp.concatenate([cq[2 * s], cq[2 * s + 1]], axis=1)
            x1 = x_v[pl.ds(r0 + s * HM, HM), :].astype(F32) + mod(2) * a
            x1s.append(x1)
            h2s.append(_ln_norm(x1) * mod(4) + mod(3))
        sops = [u.astype(BF16) for u in
                _a_ops(h2s[0][:, 0:NH], h2s[0][:, NH:], h2s[1][:, 0:NH], h2s[1][:, NH:])]
        accs = [None] * 7
        blk = 0
        for f in range(NCH):
            fs = slice(f * SN, (f + 1) * SN)
            g = _c_quads([_dot(sops[p], _bf(w1_v[p, :, fs])) for p in range(7)])
            u = _c_quads([_dot(sops[p], _bf(w3_v[p, :, fs])) for p in range(7)])
            act = []
            for gg, uu in zip(g, u):
                hg = 0.5 * gg
                act.append((hg + hg * jnp.tanh(hg)) * uu)
            aops = [v.astype(BF16) for v in _a_ops(*act)]
            for _ in range(SCH[f]):
                attn_block(pl.multiple_of(
                    jnp.minimum((i + 1) * NBLK + blk, S // RB - 1) * RB, RB), False)
                blk += 1
            for p in range(7):
                t = _dot(aops[p], _bf(w2_v[p, f * SN // 2:(f + 1) * SN // 2, :]))
                accs[p] = t if accs[p] is None else accs[p] + t
        c11, c12, c21, c22 = _c_quads(accs)
        g5 = mod(5)
        o_v[pl.ds(r0, HM), 0:NH] = (x1s[0][:, 0:NH] + g5[:, 0:NH] * c11).astype(BF16)
        o_v[pl.ds(r0, HM), NH:] = (x1s[0][:, NH:] + g5[:, NH:] * c12).astype(BF16)
        o_v[pl.ds(r0 + HM, HM), 0:NH] = (x1s[1][:, 0:NH] + g5[:, 0:NH] * c21).astype(BF16)
        o_v[pl.ds(r0 + HM, HM), NH:] = (x1s[1][:, NH:] + g5[:, NH:] * c22).astype(BF16)
        out_copy(r0).start()
        return carry

    lax.fori_loop(0, NT, body_b, 0)
    for i in range(NT):
        out_copy(i * TM).wait()


@jax.jit
def pallas_adaLN_cond__sliding_local_dilated__glu_gated_swiglu__prompt_kernel(
    A_x: jax.Array,
    A_wqkv: jax.Array,
    A_wo: jax.Array,
    B_x: jax.Array,
    B_w1: jax.Array,
    B_w3: jax.Array,
    B_w2: jax.Array,
    c: jax.Array,
    w_mod: jax.Array,
):
    del B_x
    anyspec = pl.BlockSpec(memory_space=pl.ANY)
    out = pl.pallas_call(
        _kernel,
        in_specs=[anyspec] * 8,
        out_specs=anyspec,
        out_shape=jax.ShapeDtypeStruct((S, D), BF16),
        scratch_shapes=[
            pltpu.VMEM((S, D), BF16),
            pltpu.VMEM((1, D), BF16),
            pltpu.VMEM((4, 4, QR, NH), U32),
            pltpu.VMEM((4, 4, QR, NH), U32),
            pltpu.VMEM((7, D // 4, F // 2), U32),
            pltpu.VMEM((7, D // 4, F // 2), U32),
            pltpu.VMEM((7, F // 4, D // 2), U32),
            pltpu.VMEM((6, D // 2, D), U32),
            pltpu.VMEM((6, 16, D), F32),
            pltpu.VMEM((3, 8, D), F32),
            pltpu.VMEM((S // 2, D), U32),
            pltpu.VMEM((NSL, S + HALO, 128), F32),
            pltpu.VMEM((NSL, S + HALO, 128), F32),
            pltpu.VMEM((7, T1 // 4, NH), U32),
            pltpu.VMEM((4, T0 // 4, NH), U32),
            pltpu.VMEM((4, T0 // 4, NH), U32),
            pltpu.VMEM((S // 2, D), U32),
            pltpu.VMEM((S, D), BF16),
            pltpu.SemaphoreType.DMA((28,)),
            pltpu.SemaphoreType.DMA(()),
        ],
        compiler_params=pltpu.CompilerParams(
            vmem_limit_bytes=120 * 1024 * 1024,
            flags={"XLA_TPU_EVENLY_DISTRIBUTE_CRITICAL_NODES": True}),
    )(A_x.reshape(S, D), c, A_wqkv, A_wo, B_w1, B_w3, B_w2, w_mod)
    return out.reshape(1, S, D)
```
